```python
import jax
import jax.numpy as jnp

def _softmax(x, axis=-1):
    return jax.nn.softmax(x, axis=axis)

def _gelu(x):
    return jax.nn.gelu(x, approximate=True)

def _silu(x):
    return jax.nn.silu(x)

def _sigmoid(x):
    return jax.nn.sigmoid(x)

def _layernorm(x, axis=-1, eps=1e-05):
    m = jnp.mean(x, axis=axis, keepdims=True)
    v = jnp.var(x, axis=axis, keepdims=True)
    return (x - m) / jnp.sqrt(v + eps)

def _scatter_add(tgt, idx, src, axis=0):
    return tgt.at[idx].add(src)

def _segment_sum(src, seg, n):
    return jax.ops.segment_sum(src, seg, n)

class _Rng:

    def __init__(self, key):
        self._k = key

    def _next(self):
        self._k, sub = jax.random.split(self._k)
        return sub

    def normal(self, shape):
        return jax.random.normal(self._next(), shape, dtype=jnp.bfloat16)

    def randint(self, lo, hi, shape):
        return jax.random.randint(self._next(), shape, lo, hi, dtype=jnp.int32)

    def uniform(self, shape, lo=0.0, hi=1.0):
        return jax.random.uniform(self._next(), shape, jnp.bfloat16, lo, hi)

    def permutation(self, n):
        return jax.random.permutation(self._next(), n)
kernel_name = 'concat_heads__memory_aug_recurrent_mem_tr__ssm_conv_h3__prompt'

def setup_inputs():
    _rng = _Rng(jax.random.key(int.from_bytes(__import__("os").urandom(4), "little")))
    _w = lambda a: (lambda t: t.astype(jnp.bfloat16) if jnp.issubdtype(t.dtype, jnp.floating) else t)(jnp.asarray(a))

    def _A_setup():
        B, S, Dm = (1, 2048, 1024)
        H, Dh = (32, 128)
        M, seg = (8, 32)
        seg = min(seg, S)
        S = S // seg * seg
        return {'x': _w((lambda *s: _rng.normal(s) * 0.05)(B, S, Dm)), 'mem0': _w((lambda *s: _rng.normal(s) * 0.05)(B, M, Dm)), 'Wq': _w((lambda *s: _rng.normal(s) * 0.05)(Dm, H, Dh) * Dm ** (-0.5)), 'Wk': _w((lambda *s: _rng.normal(s) * 0.05)(Dm, H, Dh) * Dm ** (-0.5)), 'Wv': _w((lambda *s: _rng.normal(s) * 0.05)(Dm, H, Dh) * Dm ** (-0.5)), 'Wo': _w((lambda *s: _rng.normal(s) * 0.05)(H, Dh, Dm) * (H * Dh) ** (-0.5)), 'seg_len': seg}
    _A_in = _A_setup()

    def _B_setup():
        B, S, D = (1, 2048, 1024)
        ks = 4
        return {'q': _w((lambda *s: _rng.normal(s) * 0.05)(B, S, D)), 'k': _w((lambda *s: _rng.normal(s) * 0.05)(B, S, D)), 'v': _w((lambda *s: _rng.normal(s) * 0.05)(B, S, D)), 'shift_k': _w((lambda *s: _rng.normal(s) * 0.05)(D, ks) * 0.5), 'ssm_k': _w((lambda *s: _rng.normal(s) * 0.05)(D, S) * (1.0 / S ** 0.5)), 'ssm_D': _w((lambda *s: _rng.normal(s) * 0.05)(D))}
    _B_in = _B_setup()
    return {'A_x': _A_in['x'], 'A_mem0': _A_in['mem0'], 'A_Wq': _A_in['Wq'], 'A_Wk': _A_in['Wk'], 'A_Wv': _A_in['Wv'], 'A_Wo': _A_in['Wo'], 'A_seg_len': _A_in['seg_len'], 'B_q': _B_in['q'], 'B_k': _B_in['k'], 'B_v': _B_in['v'], 'B_shift_k': _B_in['shift_k'], 'B_ssm_k': _B_in['ssm_k'], 'B_ssm_D': _B_in['ssm_D']}

def reference(A_x, A_mem0, A_Wq, A_Wk, A_Wv, A_Wo, A_seg_len, B_q, B_k, B_v, B_shift_k, B_ssm_k, B_ssm_D):

    def _A_ref(x, mem0, Wq, Wk, Wv, Wo, seg_len):
        B, S, Dm = x.shape
        H, Dh = (Wq.shape[1], Wq.shape[2])
        M = mem0.shape[1]
        scale = Dh ** (-0.5)
        n_seg = S // seg_len
        L = M + seg_len
        idx = jnp.arange(L)
        mask = (idx[:, None] < M) | (idx[:, None] >= idx[None, :])
        mem = mem0
        outs = []
        for s in range(n_seg):
            xs = x[:, s * seg_len:(s + 1) * seg_len, :].copy()
            h = jnp.concatenate([mem, xs], axis=1)
            q = jnp.einsum('btd,dhe->bhte', h, Wq)
            k = jnp.einsum('btd,dhe->bhte', h, Wk)
            v = jnp.einsum('btd,dhe->bhte', h, Wv)
            scores = jnp.einsum('bhqe,bhke->bhqk', q, k) * scale
            scores = jnp.where(mask[None, None], scores, -1000000000.0)
            p = _softmax(scores, axis=-1)
            o = jnp.einsum('bhqk,bhke->bhqe', p, v)
            o = jnp.einsum('bhte,hed->btd', o, Wo)
            mem = o[:, :M, :].copy()
            outs.append(o[:, M:, :])
        return jnp.concatenate(outs, axis=1)

    def _B_ref(q, k, v, shift_k, ssm_k, ssm_D):
        B, S, D = q.shape
        ks = shift_k.shape[-1]
        k_pad = jnp.pad(k, ((0, 0), (ks - 1, 0), (0, 0)))
        k_shift = jnp.zeros_like(k)
        for t in range(ks):
            k_shift = k_shift + k_pad[:, t:t + S, :] * shift_k[:, ks - 1 - t][None, None, :]
        kv = k_shift * v
        L = 2 * S
        kv_pad = jnp.pad(kv, ((0, 0), (0, S), (0, 0)))
        kf_pad = jnp.pad(ssm_k, ((0, 0), (0, S)))
        kv_f = (lambda x, axes=(-2, -1): jnp.fft.rfft2(x.astype(jnp.float32), axes=axes))(kv_pad[:, None, :, :], axes=(1, 2))
        kf_f = (lambda x, axes=(-2, -1): jnp.fft.rfft2(x.astype(jnp.float32), axes=axes))(kf_pad[:, None, :], axes=(1, 2))
        kf_f = (lambda x, *d: x.transpose(*d))(kf_f, 1, 2, 0)
        y_f = kv_f * kf_f[None, :, :, :]
        y = (lambda x, s, axes=(-2, -1): jnp.fft.irfft2(x, s=s, axes=axes).astype(jnp.bfloat16))(y_f, (1, L), axes=(1, 2))[:, 0, :S, :]
        y = y + kv * ssm_D[None, None, :]
        return q * y
    a = _A_ref(A_x, A_mem0, A_Wq, A_Wk, A_Wv, A_Wo, A_seg_len)
    b = _B_ref(B_q, B_k, B_v, B_shift_k, B_ssm_k, B_ssm_D)
    return jnp.concatenate([a, b], axis=-1)
```

```python
import functools

import jax
import jax.numpy as jnp
import numpy as np
import jax.experimental.pallas as pl
import jax.experimental.pallas.tpu as pltpu

BF16 = jnp.bfloat16
F32 = jnp.float32
U32 = jnp.uint32

LANES = 128
CHUNK = 128


def _dft_tables():
    n = np.arange(CHUNK, dtype=np.float64)
    f = np.concatenate([np.arange(0, CHUNK, 2), np.arange(1, CHUNK, 2)]).astype(np.float64)
    theta = 2.0 * np.pi * (f[:, None] + 0.5) * n[None, :] / (2 * CHUNK)
    fwd = np.concatenate([np.cos(theta), -np.sin(theta)], axis=0)
    inv = np.concatenate([np.cos(theta).T, -np.sin(theta).T], axis=1) / CHUNK
    return fwd.astype(np.float32), inv.astype(np.float32)


_FWD, _INV = _dft_tables()


def _kernel(
    mem_ref, shift_ref, dvec_ref, fwd_ref, inv_ref,
    x_hbm, wq_hbm, wk_hbm, wv_hbm, wo_hbm, bq_hbm, bk_hbm, bv_hbm, ssm_hbm,
    out_hbm,
    wqkv, wo, stage, xbuf, abuf, hbuf,
    qb, kb, vb, sb, kf, kvb, xs, ks, ys, ob,
    sem_w, sem_wo, sem_x, sem_in, sem_ob, sem_a,
    *, S, DM, H, E, M, SEG, D, KS,
):
    L = M + SEG
    NSEG = S // SEG
    NCT = D // LANES
    NCH = S // CHUNK
    DCH = DM // NCT
    HP = H // 2
    NT = DM // LANES

    wq32 = wq_hbm.bitcast(U32)
    wk32 = wk_hbm.bitcast(U32)
    wv32 = wv_hbm.bitcast(U32)
    wo32 = wo_hbm.bitcast(U32)

    def b_in_copies(c, slot):
        col = pl.ds(pl.multiple_of(c * LANES, LANES), LANES)
        return (
            pltpu.make_async_copy(bk_hbm.at[:, col], kb.at[slot], sem_in.at[slot, 0]),
            pltpu.make_async_copy(bv_hbm.at[:, col], vb.at[slot], sem_in.at[slot, 1]),
            pltpu.make_async_copy(ssm_hbm.at[col, :], sb.at[slot], sem_in.at[slot, 2]),
            pltpu.make_async_copy(bq_hbm.at[:, col], qb.at[slot], sem_in.at[slot, 3]),
        )

    def w_copies(c, slot):
        rows = pl.ds(pl.multiple_of(c * DCH * HP, DCH * HP), DCH * HP)
        return tuple(
            pltpu.make_async_copy(w.at[rows, :], stage.at[slot, i], sem_w.at[slot, i])
            for i, w in enumerate((wq32, wk32, wv32))
        )

    def wo_copy(n):
        col = pl.ds(pl.multiple_of(n * LANES, LANES), LANES)
        return pltpu.make_async_copy(wo32.at[:, col], wo.at[n], sem_wo)

    def ob_copy(c, slot):
        col = pl.ds(pl.multiple_of(DM + c * LANES, LANES), LANES)
        return pltpu.make_async_copy(ob.at[slot], out_hbm.at[:, col], sem_ob.at[slot])

    x_copy = pltpu.make_async_copy(x_hbm, xbuf, sem_x)

    def relayout(c, slot):
        r0 = pl.multiple_of(c * (DCH // 2), DCH // 2)
        for i in range(3):
            for j in range(HP):
                for dd in range(DCH // 16):
                    a = stage[slot, i, pl.ds(dd * 16 * HP + j, 8, stride=2 * HP), :]
                    b = stage[slot, i, pl.ds(dd * 16 * HP + HP + j, 8, stride=2 * HP), :]
                    lo = (a & jnp.uint32(0xFFFF)) | (b << 16)
                    hi = (a >> 16) | (b & jnp.uint32(0xFFFF0000))
                    wqkv[3 * (2 * j) + i, pl.ds(r0 + dd * 8, 8), :] = lo
                    wqkv[3 * (2 * j + 1) + i, pl.ds(r0 + dd * 8, 8), :] = hi

    def b_tile(c, slot):
        col0 = pl.multiple_of(c * LANES, LANES)
        sh = shift_ref[pl.ds(col0, LANES), :]
        sel = (jax.lax.broadcasted_iota(jnp.int32, (8, KS), 0)
               == jax.lax.broadcasted_iota(jnp.int32, (8, KS), 1)).astype(BF16)
        taps = jax.lax.dot_general(sel, sh, (((1,), (1,)), ((), ())),
                                   preferred_element_type=F32)
        dvec = dvec_ref[:, pl.ds(col0, LANES)].astype(F32)

        kf[0:8, :] = jnp.zeros((8, LANES), F32)
        kf[8:, :] = kb[slot].astype(F32)

        fwd = fwd_ref[...]
        half = CHUNK // 2

        def dft_chunk(j, prev):
            t0 = pl.multiple_of(j * CHUNK, CHUNK)
            acc = kf[pl.ds(t0 + 8, CHUNK), :] * taps[0:1, :]
            for t in range(1, KS):
                acc = acc + kf[pl.ds(t0 + 8 - t, CHUNK), :] * taps[t:t + 1, :]
            kv = (acc * vb[slot, pl.ds(t0, CHUNK), :].astype(F32)).astype(BF16)
            kvb[pl.ds(t0, CHUNK), :] = kv
            kspec = jax.lax.dot_general(fwd, sb[slot, :, pl.ds(t0, CHUNK)],
                                        (((1,), (1,)), ((), ())), preferred_element_type=F32)
            ks[j] = kspec
            xj = jnp.dot(fwd, kv, preferred_element_type=F32)
            pre_e, pre_o = xs[j, 0:half, :], xs[j, half:CHUNK, :]
            pim_e, pim_o = xs[j, CHUNK:CHUNK + half, :], xs[j, CHUNK + half:, :]
            xs[j + 1] = xj
            xs[j, 0:half, :] = xj[0:half] - pim_e
            xs[j, half:CHUNK, :] = xj[half:CHUNK] + pim_o
            xs[j, CHUNK:CHUNK + half, :] = xj[CHUNK:CHUNK + half] + pre_e
            xs[j, CHUNK + half:, :] = xj[CHUNK + half:] - pre_o
            return prev

        xs[0] = jnp.zeros((2 * CHUNK, LANES), F32)
        jax.lax.fori_loop(0, NCH, dft_chunk, 0)

        def products(fb, carry):
            r = pl.multiple_of(fb * 8, 8)
            re = pl.ds(r, 8)
            im = pl.ds(r + CHUNK, 8)
            grp = 4
            for ig in range(NCH // grp):
                accs = [None] * grp
                xv = {}
                for m in range(grp * ig + grp):
                    kr = ks[m, re, :]
                    ki = ks[m, im, :]
                    for u in range(grp):
                        j = grp * ig + u - m
                        if j < 0:
                            continue
                        if j not in xv:
                            xv[j] = (xs[j, re, :], xs[j, im, :])
                        xr, xi = xv[j]
                        if accs[u] is None:
                            accs[u] = (kr * xr - ki * xi, kr * xi + ki * xr)
                        else:
                            ar, ai = accs[u]
                            accs[u] = (ar + kr * xr - ki * xi, ai + kr * xi + ki * xr)
                for u in range(grp):
                    ys[grp * ig + u, re, :] = accs[u][0]
                    ys[grp * ig + u, im, :] = accs[u][1]
            return carry

        jax.lax.fori_loop(0, CHUNK // 8, products, 0)

        @pl.when(c >= 2)
        def _():
            ob_copy(c - 2, slot).wait()

        inv = inv_ref[...]

        def inverse(i, carry):
            t0 = pl.multiple_of(i * CHUNK, CHUNK)
            y = jnp.dot(inv, ys[i].astype(BF16), preferred_element_type=F32)
            rows = pl.ds(t0, CHUNK)
            kv = kvb[rows, :].astype(F32)
            qv = qb[slot, rows, :].astype(F32)
            ob[slot, rows, :] = (qv * (y + kv * dvec)).astype(BF16)
            return carry

        jax.lax.fori_loop(0, NCH, inverse, 0)
        ob_copy(c, slot).start()

    for cp in b_in_copies(0, 0):
        cp.start()
    for cp in w_copies(0, 0):
        cp.start()

    def b_iter(c, carry):
        slot = jax.lax.rem(c, 2)
        nxt = 1 - slot

        @pl.when(c + 1 < NCT)
        def _():
            for cp in b_in_copies(c + 1, nxt):
                cp.start()
            for cp in w_copies(c + 1, nxt):
                cp.start()

        wo_copy(c).start()

        @pl.when(c + 1 == NCT)
        def _():
            x_copy.start()

        for cp in b_in_copies(c, slot):
            cp.wait()
        b_tile(c, slot)
        for cp in w_copies(c, slot):
            cp.wait()
        relayout(c, slot)
        return carry

    jax.lax.fori_loop(0, NCT, b_iter, 0)

    pltpu.make_async_copy(wo, wo, sem_wo).wait()
    x_copy.wait()

    row = jax.lax.broadcasted_iota(jnp.int32, (L, L), 0)
    col = jax.lax.broadcasted_iota(jnp.int32, (L, L), 1)
    mask = (row < M) | (row >= col)
    scale = E ** -0.5
    hbuf[0:M, :] = mem_ref[...].astype(F32)

    def wt(i):
        return pltpu.bitcast(wqkv[i], BF16)

    def segment(s, carry):
        r0 = pl.multiple_of(s * SEG, SEG)
        hbuf[M:L, :] = xbuf[pl.ds(r0, SEG), :].astype(F32)
        h = hbuf[...]
        Q, K, V, P, O = {}, {}, {}, {}, {}
        acc = [None] * NT

        def scores(hd):
            sc = jax.lax.dot_general(Q.pop(hd), K.pop(hd), (((1,), (1,)), ((), ())),
                                     preferred_element_type=F32)
            sc = jnp.where(mask, sc * scale, -1e9)
            mx = jnp.max(sc, axis=-1, keepdims=True)
            p = jnp.exp(sc - mx)
            P[hd] = p / jnp.sum(p, axis=-1, keepdims=True)

        def values(hd):
            O[hd] = jnp.dot(P.pop(hd), V.pop(hd), preferred_element_type=F32)

        def project(hd):
            o = O.pop(hd)
            for n in range(NT):
                w = pltpu.bitcast(wo[n, hd * (E // 2):(hd + 1) * (E // 2), :], BF16)
                y = jnp.dot(o, w, preferred_element_type=F32)
                acc[n] = y if acc[n] is None else acc[n] + y

        for t in range(H + 4):
            if t < H:
                Q[t] = jnp.dot(h, wt(3 * t), preferred_element_type=F32)
            if 0 <= t - 1 < H:
                scores(t - 1)
            if t < H:
                K[t] = jnp.dot(h, wt(3 * t + 1), preferred_element_type=F32).astype(BF16)
            if 0 <= t - 2 < H:
                values(t - 2)
            if t < H:
                V[t] = jnp.dot(h, wt(3 * t + 2), preferred_element_type=F32).astype(BF16)
            if 0 <= t - 3 < H:
                project(t - 3)
        out = jnp.concatenate(acc, axis=1).astype(BF16)
        hbuf[0:M, :] = out[0:M].astype(F32)
        abuf[pl.ds(r0, SEG), :] = out[M:L]
        pltpu.make_async_copy(
            abuf.at[pl.ds(r0, SEG), :], out_hbm.at[pl.ds(r0, SEG), pl.ds(0, DM)], sem_a
        ).start()
        return carry

    jax.lax.fori_loop(0, NSEG, segment, 0)

    ob_copy(NCT - 2, (NCT - 2) % 2).wait()
    ob_copy(NCT - 1, (NCT - 1) % 2).wait()
    pltpu.make_async_copy(abuf, out_hbm.at[:, pl.ds(0, DM)], sem_a).wait()


@functools.partial(jax.jit, static_argnames=("A_seg_len",))
def pallas_concat_heads__memory_aug_recurrent_mem_tr__ssm_conv_h3__prompt_kernel(
    A_x: jax.Array,
    A_mem0: jax.Array,
    A_Wq: jax.Array,
    A_Wk: jax.Array,
    A_Wv: jax.Array,
    A_Wo: jax.Array,
    A_seg_len: int,
    B_q: jax.Array,
    B_k: jax.Array,
    B_v: jax.Array,
    B_shift_k: jax.Array,
    B_ssm_k: jax.Array,
    B_ssm_D: jax.Array,
):
    B, S, DM = A_x.shape
    H, E = A_Wq.shape[1], A_Wq.shape[2]
    M = A_mem0.shape[1]
    SEG = int(A_seg_len)
    D = B_q.shape[2]
    KS = B_shift_k.shape[1]
    assert B == 1 and E == LANES and S % CHUNK == 0 and S % SEG == 0
    NCT = D // LANES
    NCH = S // CHUNK
    DCH = DM // NCT

    kernel = functools.partial(_kernel, S=S, DM=DM, H=H, E=E, M=M, SEG=SEG, D=D, KS=KS)
    vmem = pl.BlockSpec(memory_space=pltpu.VMEM)
    hbm = pl.BlockSpec(memory_space=pl.ANY)
    dma = pltpu.SemaphoreType.DMA

    out = pl.pallas_call(
        kernel,
        out_shape=jax.ShapeDtypeStruct((S, DM + D), BF16),
        in_specs=[vmem] * 5 + [hbm] * 9,
        out_specs=hbm,
        scratch_shapes=[
            pltpu.VMEM((3 * H, DM // 2, E), U32),
            pltpu.VMEM((DM // LANES, H * E // 2, LANES), U32),
            pltpu.VMEM((2, 3, DCH * (H // 2), E), U32),
            pltpu.VMEM((S, DM), BF16),
            pltpu.VMEM((S, DM), BF16),
            pltpu.VMEM((M + SEG, DM), F32),
            pltpu.VMEM((2, S, LANES), BF16),
            pltpu.VMEM((2, S, LANES), BF16),
            pltpu.VMEM((2, S, LANES), BF16),
            pltpu.VMEM((2, LANES, S), BF16),
            pltpu.VMEM((8 + S, LANES), F32),
            pltpu.VMEM((S, LANES), BF16),
            pltpu.VMEM((NCH + 1, 2 * CHUNK, LANES), F32),
            pltpu.VMEM((NCH, 2 * CHUNK, LANES), F32),
            pltpu.VMEM((NCH, 2 * CHUNK, LANES), F32),
            pltpu.VMEM((2, S, LANES), BF16),
            dma((2, 3)), dma, dma, dma((2, 4)), dma((2,)), dma,
        ],
        compiler_params=pltpu.CompilerParams(vmem_limit_bytes=120 * 1024 * 1024),
    )(
        A_mem0.reshape(M, DM), B_shift_k, B_ssm_D.reshape(1, D),
        jnp.asarray(_FWD, BF16), jnp.asarray(_INV, BF16),
        A_x.reshape(S, DM),
        A_Wq.reshape(DM * H, E), A_Wk.reshape(DM * H, E), A_Wv.reshape(DM * H, E),
        A_Wo.reshape(H * E, DM),
        B_q.reshape(S, D), B_k.reshape(S, D), B_v.reshape(S, D), B_ssm_k,
    )
    return out.reshape(B, S, DM + D)
```

```python
import functools

DBG = frozenset(('tp1=6', 'nfree=10'))

import jax
import jax.numpy as jnp
import numpy as np
import jax.experimental.pallas as pl
import jax.experimental.pallas.tpu as pltpu

BF16 = jnp.bfloat16
F32 = jnp.float32
U32 = jnp.uint32

LANES = 128
LOG2E = 1.4426950408889634
CHUNK = 128


def _dft_tables():
    n = np.arange(CHUNK, dtype=np.float64)
    f = np.concatenate([np.arange(0, CHUNK, 2), np.arange(1, CHUNK, 2)]).astype(np.float64)
    theta = 2.0 * np.pi * (f[:, None] + 0.5) * n[None, :] / (2 * CHUNK)
    fwd = np.concatenate([np.cos(theta), -np.sin(theta)], axis=0)
    inv = np.concatenate([np.cos(theta).T, -np.sin(theta).T], axis=1) / CHUNK
    return fwd.astype(np.float32), inv.astype(np.float32)


_FWD, _INV = _dft_tables()


def _opt(name, default):
    for tok in DBG:
        if tok.startswith(name + "="):
            v = tok[len(name) + 1:]
            return int(v) if v.lstrip("-").isdigit() else v
    return default


def _mult(x, n):
    return x if isinstance(x, int) else pl.multiple_of(x, n)


def _rem(x, n):
    return x % n if isinstance(x, int) else jax.lax.rem(x, n)


NSLOT = 3


def _kernel(
    mem_hbm, shift_hbm, dvec_hbm, fwd_hbm, inv_hbm,
    x_hbm, wq_hbm, wk_hbm, wv_hbm, wo_hbm, bq_hbm, bk_hbm, bv_hbm, ssm_hbm,
    out_hbm,
    arena, wo, stage, xbuf, abuf, hbuf, accb,
    qb, kb, vb, sb, kf, xraw, xs, ks, ysf,
    mem_ref, shift_ref, dvec_ref, fwd_ref, inv_ref, sem_s, dvf,
    sem_w, sem_wo, sem_x, sem_q, sem_in, sem_ob, sem_a,
    *, S, DM, H, E, M, SEG, D, KS,
):
    L = M + SEG
    NSEG = S // SEG
    NCT = D // LANES
    NCH = S // CHUNK
    DCH = DM // NCT
    HP = H // 2
    NT = DM // LANES
    SPT = NSEG // NCT
    FPS = (CHUNK // 8) // SPT
    CPS = NCH // SPT
    XR = S // NCT
    TR = DM // 2
    SPEC = 2 * CHUNK
    NSP = NCH * SPEC // TR
    YS0 = 3 * H

    wq32 = wq_hbm.bitcast(U32)
    wk32 = wk_hbm.bitcast(U32)
    wv32 = wv_hbm.bitcast(U32)

    def lanes_of(c):
        return pl.ds(_mult(c * LANES, LANES), LANES)

    def b_in_copies(c):
        col = lanes_of(c)
        return (
            pltpu.make_async_copy(bk_hbm.at[:, col], kb.at[:, col], sem_in.at[c, 0]),
            pltpu.make_async_copy(bv_hbm.at[:, col], vb.at[:, col], sem_in.at[c, 1]),
            pltpu.make_async_copy(ssm_hbm.at[col, :], sb.at[col, :], sem_in.at[c, 2]),
        )

    def w_copies(c, slot):
        rows = pl.ds(_mult(c * DCH * HP, DCH * HP), DCH * HP)
        return tuple(
            pltpu.make_async_copy(w.at[rows, :], stage.at[slot, i], sem_w.at[slot, i])
            for i, w in enumerate((wq32, wk32, wv32))
        )

    WO32 = False

    def wo_copy(p):
        rows = pl.ds(_mult(p * (H * E // NCT), H * E // NCT), H * E // NCT)
        return pltpu.make_async_copy(wo_hbm.at[rows, :], wo.at[rows, :], sem_wo.at[p])

    def late_copies(c):
        rows = pl.ds(_mult(c * XR, XR), XR)
        return (
            pltpu.make_async_copy(x_hbm.at[rows, :], xbuf.at[rows, :], sem_x.at[c]),
            pltpu.make_async_copy(bq_hbm.at[:, lanes_of(c)], qb.at[:, lanes_of(c)], sem_q.at[c]),
        )

    def ob_copy(c, part):
        n = CPS * CHUNK
        rows = pl.ds(_mult(part * n, n), n)
        return pltpu.make_async_copy(qb.at[rows, lanes_of(c)], out_hbm.at[rows, lanes_of(NT + c)], sem_ob)

    def spec_rows(base, slot, j, r, n):
        tile = base + slot * NSP + j // (TR // SPEC)
        row = _mult((j % (TR // SPEC)) * SPEC + r, 8)
        return tile, pl.ds(row, n)

    def spec_load(base, slot, j, r, n):
        tile, rows = spec_rows(base, slot, j, r, n)
        return pltpu.bitcast(arena[tile, rows, :], F32)

    def spec_store(base, slot, j, r, val):
        tile, rows = spec_rows(base, slot, j, r, val.shape[0])
        arena[tile, rows, :] = pltpu.bitcast(val, U32)

    def relayout(c, slot, i):
        r0 = _mult(c * (DCH // 2), DCH // 2)

        def repack(words):
            return pltpu.bitcast(pltpu.bitcast(words, F32).astype(BF16), U32)

        if True:
            for j in range(HP):
                for dd in range(DCH // 16):
                    a = stage[slot, i, pl.ds(dd * 16 * HP + j, 8, stride=HP), :]
                    b = stage[slot, i, pl.ds((dd * 16 + 8) * HP + j, 8, stride=HP), :]
                    ab = jnp.concatenate([a, b], axis=0)
                    dst = pl.ds(r0 + dd * 8, 8)
                    arena[3 * (2 * j) + i, dst, :] = repack(ab << 16)
                    arena[3 * (2 * j + 1) + i, dst, :] = repack(ab & jnp.uint32(0xFFFF0000))

    def conv_taps(c):
        return shift_ref[:, lanes_of(c)].astype(F32)

    def stage_k(c, part):
        n = CPS * CHUNK
        kf[0:8, :] = jnp.where(part == 0, 0.0, kf[n:n + 8, :])
        kf[8:n + 8, :] = kb[pl.ds(_mult(part * n, n), n), lanes_of(c)].astype(F32)

    KVP = _opt("kvp", 4)

    def kv_piece(c, part, u, taps, piece):
        n = CHUNK // KVP
        j = part * CPS + u
        rows = pl.ds(_mult(j * CHUNK + piece * n, n), n)
        k0 = u * CHUNK + piece * n + 8
        acc = kf[k0:k0 + n, :] * taps[0:1, :]
        for t in range(1, KS):
            acc = acc + kf[k0 - t:k0 - t + n, :] * taps[t:t + 1, :]
        kv = (acc * vb[rows, lanes_of(c)].astype(F32)).astype(BF16)
        vb[rows, lanes_of(c)] = kv
        return kv

    def kv_chunk(c, part, u, taps):
        return jnp.concatenate([kv_piece(c, part, u, taps, q) for q in range(KVP)], axis=0)

    def x_spectrum(slot, part, u, kv):
        j = part * CPS + u
        half = CHUNK // 2
        xj = jnp.dot(fwd_ref[...], kv, preferred_element_type=F32)
        prev = xraw[u % 2]
        if u == 0:
            prev = jnp.where(part == 0, 0.0, prev)
        xraw[1 - u % 2] = xj
        xs[slot, j, 0:half, :] = xj[0:half] - prev[CHUNK:CHUNK + half]
        xs[slot, j, half:CHUNK, :] = xj[half:CHUNK] + prev[CHUNK + half:]
        xs[slot, j, CHUNK:CHUNK + half, :] = xj[CHUNK:CHUNK + half] + prev[0:half]
        xs[slot, j, CHUNK + half:, :] = xj[CHUNK + half:] - prev[half:CHUNK]

    def k_spectrum(c, slot, part, u):
        j = part * CPS + u
        blk = sb[lanes_of(c), pl.ds(_mult(j * CHUNK, CHUNK), CHUNK)]
        ks[slot, j] = jax.lax.dot_general(
            fwd_ref[...], blk, (((1,), (1,)), ((), ())), preferred_element_type=F32)

    GRP = _opt("grp", 2)

    def products(slot, fb, ig, free):
        r = _mult(fb * 8, 8)
        re, im = pl.ds(r, 8), pl.ds(r + CHUNK, 8)
        accs = [None] * GRP
        xv = {}
        for m in range(GRP * ig + GRP):
            kr = ks[slot, m, re, :]
            ki = ks[slot, m, im, :]
            for u in range(GRP):
                j = GRP * ig + u - m
                if j < 0:
                    continue
                if j not in xv:
                    xv[j] = (xs[slot, j, re, :], xs[slot, j, im, :])
                xr, xi = xv[j]
                if accs[u] is None:
                    accs[u] = (kr * xr - ki * xi, kr * xi + ki * xr)
                else:
                    ar, ai = accs[u]
                    accs[u] = (ar + kr * xr - ki * xi, ai + kr * xi + ki * xr)
            yield
        for u in range(GRP):
            if free:
                ysf[slot, GRP * ig + u, re, :] = accs[u][0]
                ysf[slot, GRP * ig + u, im, :] = accs[u][1]
            else:
                spec_store(YS0, slot, GRP * ig + u, r, accs[u][0])
                spec_store(YS0, slot, GRP * ig + u, r + CHUNK, accs[u][1])

    NFREE = _opt("nfree", 8)

    def is_free(f, ig):
        return f * (NCH // GRP) + ig >= NFREE

    def y_load(slot, i):
        pieces = []
        for blk in range(SPEC // 8):
            f = (blk % (CHUNK // 8)) % FPS
            pieces.append(lambda ig, blk=blk, f=f: None)
        return None

    def inverse(c, slot, i):
        cols = lanes_of(c)
        rows = pl.ds(_mult(i * CHUNK, CHUNK), CHUNK)
        dvec = dvf[pl.ds(c, 1), :]
        ya = spec_load(YS0, slot, i, 0, SPEC)
        yb = ysf[slot, i]
        yy = jnp.concatenate([(yb if is_free((blk % (CHUNK // 8)) % FPS, 0) else ya)[blk * 8:blk * 8 + 8]
                              for blk in range(SPEC // 8)], axis=0)
        y = jnp.dot(inv_ref[...], yy.astype(BF16), preferred_element_type=F32)
        kv = vb[rows, cols].astype(F32)
        qv = qb[rows, cols].astype(F32)
        qb[rows, cols] = (qv * (y + kv * dvec)).astype(BF16)

    def spectra_part(c, slot, part, taps):
        stage_k(c, part)
        for u in range(CPS):
            x_spectrum(slot, part, u, kv_chunk(c, part, u, taps))
            k_spectrum(c, slot, part, u)

    small = [pltpu.make_async_copy(a, b, sem_s.at[i]) for i, (a, b) in enumerate(
        ((mem_hbm, mem_ref), (shift_hbm, shift_ref), (dvec_hbm, dvec_ref), (fwd_hbm, fwd_ref), (inv_hbm, inv_ref)))]
    for c0 in range(NSLOT - 1):
        for cp in w_copies(c0, c0):
            cp.start()
    for cp in small:
        cp.start()
    for c0 in range(2):
        for cp in b_in_copies(c0):
            cp.start()
    for cp in late_copies(0):
        cp.start()
    for cp in small:
        cp.wait()
    dvf[...] = dvec_ref[...].astype(F32)

    def pro_iter(c, carry):
        slot = jax.lax.rem(c, NSLOT)
        ahead = c + NSLOT - 1

        @pl.when(ahead < NCT)
        def _():
            for cp in w_copies(ahead, jax.lax.rem(ahead, NSLOT)):
                cp.start()

        WOA, WOB = _opt("woa", 1), _opt("wob", 3)
        for cc, lo, hi in ((NCT - 3, 0, WOA), (NCT - 2, WOA, WOB), (NCT - 1, WOB, NCT)):
            @pl.when(c == cc)
            def _(lo=lo, hi=hi):
                if lo == 0:
                    for cp in b_in_copies(2):
                        cp.start()
                for p in range(lo, hi):
                    wo_copy(p).start()
        for i, cp in enumerate(w_copies(c, slot)):
            cp.wait()
            if 'norelay' not in DBG:
                relayout(c, slot, i)

        @pl.when((c == 2) | (c == 3))
        def _():
            for cp in b_in_copies(c - 2):
                cp.wait()
            taps = conv_taps(c - 2)
            if 'nopro_sp' not in DBG:
                jax.lax.fori_loop(0, SPT, lambda part, z: (spectra_part(c - 2, c - 2, part, taps), z)[1], 0)

        @pl.when(c == 4)
        def _():
            def body(fb, z):
                for f in range(FPS):
                    for ig in range(NCH // GRP):
                        for _ in products(0, fb * FPS + f, ig, is_free(f, ig)):
                            pass
                return z
            if 'nopro_pr' not in DBG:
                jax.lax.fori_loop(0, CHUNK // 8 // FPS, body, 0)

        return carry

    jax.lax.fori_loop(0, NCT, pro_iter, 0)

    def start_late():
        for c0 in range(1, NCT):
            for cp in late_copies(c0):
                cp.start()
            if c0 >= 3:
                for cp in b_in_copies(c0):
                    cp.start()

    PEEL = 'nopeel' not in DBG
    if not PEEL:
        for p in range(NCT):
            wo_copy(p).wait()
        start_late()

    row = jax.lax.broadcasted_iota(jnp.int32, (L, L), 0)
    col = jax.lax.broadcasted_iota(jnp.int32, (L, L), 1)
    mask = (row < M) | (row >= col)
    scale = E ** -0.5
    hbuf[0:M, :] = mem_ref[...].astype(F32)

    def wt(i):
        return pltpu.bitcast(arena[i], BF16)

    body_spec = [(w[0], int(w[1:])) for w in _opt("order", "K0_S1_Q0_P3_V1_O4").split("_")]
    maxlag = max(l for _, l in body_spec)
    ops = [(op, t - lag, t) for t in range(H + maxlag + 1) for op, lag in body_spec if 0 <= t - lag < H]

    def segment(s, carry, pos=0, first=False):
        _o = lambda name, d: _opt(name + ('_b' if pos else ''), _opt(name, d))
        c = s // SPT
        part = s % SPT

        @pl.when(part == 0)
        def _():
            for cp in late_copies(c):
                cp.wait()

            @pl.when(c + 2 < NCT)
            def _():
                for cp in b_in_copies(c + 2):
                    cp.wait()

        c2 = _rem(c + 2, NCT)
        par = _rem(c, 2)

        nslots = len(ops)
        side = {}

        def at(n, fn):
            side.setdefault(min(n, nslots), []).append(fn)

        def slot_of(t, op="O"):
            for n, (o, hd, tt) in enumerate(ops):
                if tt > t or (tt == t and o == op):
                    return n
            return nslots

        if 'noB' not in DBG:
            st = {}
            n0 = slot_of(_o("tsp", 14))
            if 'nospec' not in DBG:
              at(n0, lambda: (stage_k(c2, part), st.update(taps=conv_taps(c2))))
            for u in range(0 if 'nospec' in DBG else CPS):
                nu = slot_of(_o("tsp", 14) + 1 + u * _o("dsp", 6))
                for q in range(KVP):
                    at(nu + q * _o("kvd", 1), lambda u=u, q=q: st.update({(u, q): kv_piece(c2, part, u, st["taps"], q)}))
                nx = slot_of(_o("tsp", 14) + 2 + u * _o("dsp", 6), _o("xop", "O"))
                at(nx, lambda u=u: x_spectrum(par, part, u, jnp.concatenate(
                    [st.pop((u, q)) for q in range(KVP)], axis=0)))
                at(nx + _o("dk", 0), lambda u=u: k_spectrum(c2, par, part, u))
            for u in range(0 if 'noinv' in DBG else CPS):
                at(slot_of(_o("inv%d" % u, 32 + 2 * u), _o("iop", "O")),
                   functools.partial(inverse, c, par, part * CPS + u))

            def prod_stream(free):
                for n in range(FPS * (NCH // GRP)):
                    f, ig = n // (NCH // GRP), n % (NCH // GRP)
                    if is_free(f, ig) == free:
                        yield from products(1 - par, part * FPS + f, ig, free)
                        yield

            for free, k0, k1 in ((False, "tp0", "tp1"), (True, "tq0", "tq1")):
                gen = prod_stream(free)
                nmicro = sum(GRP * ig + GRP + 1 for f in range(FPS) for ig in range(NCH // GRP)
                             if is_free(f, ig) == free)
                p0 = slot_of(_o(k0, 30 if free else 0))
                p1 = slot_of(_o(k1, 31 if free else 13))
                for n in range(0 if 'noprod' in DBG else nmicro):
                    at(p0 + n * (p1 - p0) // nmicro, lambda gen=gen: next(gen))

        r0 = _mult(s * SEG, SEG)
        hbuf[M:L, :] = xbuf[pl.ds(r0, SEG), :].astype(F32)
        h = hbuf[...]
        Q, K, V, P, O, Z = {}, {}, {}, {}, {}, {}
        acc = [None] * NT

        for n, (op, hd, t) in enumerate(ops):
            for fn in side.pop(n, []):
                fn()
            if op == "Q":
                Q[hd] = jnp.dot(h, wt(3 * hd), preferred_element_type=F32)
            elif op == "K":
                K[hd] = jnp.dot(h, wt(3 * hd + 1), preferred_element_type=F32).astype(BF16)
            elif op == "V":
                V[hd] = jnp.dot(h, wt(3 * hd + 2), preferred_element_type=F32).astype(BF16)
            elif op == "S":
                sc = jax.lax.dot_general(Q.pop(hd), K.pop(hd), (((1,), (1,)), ((), ())),
                                         preferred_element_type=F32)
                sc = jnp.where(mask, sc, -1e9 / scale)
                p = jnp.exp2((sc - jnp.max(sc, axis=-1, keepdims=True)) * (scale * LOG2E))
                P[hd] = p
                Z[hd] = jnp.sum(p, axis=-1, keepdims=True)
            elif op == "P":
                z = Z.pop(hd)
                r = pltpu.reciprocal(z, approx=True)
                r = r * (2.0 - z * r)
                O[hd] = jnp.dot(P.pop(hd), V.pop(hd), preferred_element_type=F32) * r
            elif op == "O":
                if first and hd % (H // NCT) == 0:
                    wo_copy(hd // (H // NCT)).wait()
                    if hd == H - H // NCT:
                        start_late()
                o = O.pop(hd)
                for n in range(NT):
                    if WO32:
                        w = pltpu.bitcast(wo[n, hd * (E // 2):(hd + 1) * (E // 2), :], BF16)
                    else:
                        w = wo[hd * E:(hd + 1) * E, n * LANES:(n + 1) * LANES]
                    y = jnp.dot(o, w, preferred_element_type=F32)
                    if 'accreg' in DBG:
                        acc[n] = y if acc[n] is None else acc[n] + y
                    elif hd == 0:
                        accb[:, n * LANES:(n + 1) * LANES] = y
                    elif hd < H - 1:
                        accb[:, n * LANES:(n + 1) * LANES] += y
                    else:
                        acc[n] = accb[:, n * LANES:(n + 1) * LANES] + y
        for t in sorted(side):
            for fn in side[t]:
                fn()
        out = jnp.concatenate(acc, axis=1).astype(BF16)
        hbuf[0:M, :] = out[0:M].astype(F32)
        abuf[pl.ds(r0, SEG), :] = out[M:L]
        pltpu.make_async_copy(
            abuf.at[pl.ds(r0, SEG), :], out_hbm.at[pl.ds(r0, SEG), pl.ds(0, DM)], sem_a
        ).start()
        ob_copy(c, part).start()
        return carry

    nst = _opt("steps", NSEG)
    UNR = _opt("unr", 1)

    s0 = 0
    if PEEL and nst > 0:
        segment(0, 0, 0, first=True)
        s0 = 1
        while (nst - s0) % UNR:
            segment(s0, 0, 0)
            s0 += 1
    elif PEEL:
        for p in range(NCT):
            wo_copy(p).wait()
        start_late()

    def steps(i, carry):
        for u in range(UNR):
            segment(s0 + i * UNR + u, carry, u)
        return carry

    if 'dyn' in DBG:
        zero = (dvec_ref[0:1, :].astype(F32) * 0.0).astype(jnp.int32)
        jax.lax.fori_loop(0, (nst - s0) // UNR + jnp.max(zero), steps, 0)
    else:
        jax.lax.fori_loop(0, (nst - s0) // UNR, steps, 0)

    if 'keep' in DBG:
        z0 = jnp.max((dvec_ref[0:1, :].astype(F32) * 0.0).astype(jnp.int32))
        hbuf[0:8, 0:128] = xs[z0, z0, 0:8, :] + ks[z0, z0, 0:8, :] + spec_load(YS0, z0, z0, 0, 8)
        abuf[0:8, 0:128] = hbuf[0:8, 0:128].astype(BF16)
    if nst == NSEG:
        pltpu.make_async_copy(qb, qb, sem_ob).wait()
        pltpu.make_async_copy(abuf, out_hbm.at[:, pl.ds(0, DM)], sem_a).wait()
    else:
        nblk = -(-nst // SPT)
        for cc in range(nblk, NCT):
            for cp in late_copies(cc):
                cp.wait()
        for cc in range(max(nblk + 2, 2), NCT):
            for cp in b_in_copies(cc):
                cp.wait()
        for ss in range(nst):
            ob_copy(ss // SPT, ss % SPT).wait()
        if nst:
            pltpu.make_async_copy(abuf.at[0:nst * SEG], out_hbm.at[0:nst * SEG, pl.ds(0, DM)], sem_a).wait()


@functools.partial(jax.jit, static_argnames=("A_seg_len",))
def pallas_concat_heads__memory_aug_recurrent_mem_tr__ssm_conv_h3__prompt_kernel(
    A_x: jax.Array,
    A_mem0: jax.Array,
    A_Wq: jax.Array,
    A_Wk: jax.Array,
    A_Wv: jax.Array,
    A_Wo: jax.Array,
    A_seg_len: int,
    B_q: jax.Array,
    B_k: jax.Array,
    B_v: jax.Array,
    B_shift_k: jax.Array,
    B_ssm_k: jax.Array,
    B_ssm_D: jax.Array,
):
    B, S, DM = A_x.shape
    H, E = A_Wq.shape[1], A_Wq.shape[2]
    M = A_mem0.shape[1]
    SEG = int(A_seg_len)
    D = B_q.shape[2]
    KS = B_shift_k.shape[1]
    assert B == 1 and E == LANES and S % CHUNK == 0 and S % SEG == 0
    NCT = D // LANES
    NCH = S // CHUNK
    DCH = DM // NCT
    NSP = NCH * 2 * CHUNK // (DM // 2)
    CPS = NCH // (S // SEG // NCT)

    kernel = functools.partial(_kernel, S=S, DM=DM, H=H, E=E, M=M, SEG=SEG, D=D, KS=KS)
    vmem = pl.BlockSpec(memory_space=pltpu.VMEM)
    hbm = pl.BlockSpec(memory_space=pl.ANY)
    dma = pltpu.SemaphoreType.DMA

    out = pl.pallas_call(
        kernel,
        out_shape=jax.ShapeDtypeStruct((S, DM + D), BF16),
        in_specs=[hbm] * 14,
        out_specs=hbm,
        scratch_shapes=[
            pltpu.VMEM((3 * H + 2 * NSP, DM // 2, E), U32),
            pltpu.VMEM((H * E, DM), BF16) if True else pltpu.VMEM((DM // LANES, H * E // 2, LANES), U32),
            pltpu.VMEM((NSLOT, 3, DCH * (H // 2), E), U32),
            pltpu.VMEM((S, DM), BF16),
            pltpu.VMEM((S, DM), BF16),
            pltpu.VMEM((M + SEG, DM), F32),
            pltpu.VMEM((M + SEG, DM), F32),
            pltpu.VMEM((S, D), BF16),
            pltpu.VMEM((S, D), BF16),
            pltpu.VMEM((S, D), BF16),
            pltpu.VMEM((D, S), BF16),
            pltpu.VMEM((8 + CPS * CHUNK, LANES), F32),
            pltpu.VMEM((2, 2 * CHUNK, LANES), F32),
            pltpu.VMEM((2, NCH, 2 * CHUNK, LANES), F32),
            pltpu.VMEM((2, NCH, 2 * CHUNK, LANES), F32),
            pltpu.VMEM((2, NCH, 2 * CHUNK, LANES), F32),
            pltpu.VMEM((M, DM), BF16), pltpu.VMEM((KS, D), BF16), pltpu.VMEM((NCT, LANES), BF16),
            pltpu.VMEM((2 * CHUNK, CHUNK), BF16), pltpu.VMEM((CHUNK, 2 * CHUNK), BF16), dma((5,)),
            pltpu.VMEM((NCT, LANES), F32),
            dma((NSLOT, 3)), dma((NCT,)), dma((NCT,)), dma((NCT,)), dma((NCT, 3)), dma, dma,
        ],
        compiler_params=pltpu.CompilerParams(vmem_limit_bytes=124 * 1024 * 1024),
    )(
        A_mem0.reshape(M, DM), B_shift_k.T, B_ssm_D.reshape(NCT, LANES),
        jnp.asarray(_FWD, BF16), jnp.asarray(_INV, BF16),
        A_x.reshape(S, DM),
        A_Wq.reshape(DM * H, E), A_Wk.reshape(DM * H, E), A_Wv.reshape(DM * H, E),
        A_Wo.reshape(H * E, DM),
        B_q.reshape(S, D), B_k.reshape(S, D), B_v.reshape(S, D), B_ssm_k,
    )
    return out.reshape(B, S, DM + D)
```

```python
import functools


DBG = frozenset(('order=K0_P3_Q0_S1_V1_O4', 'grp=2', 'nfree=10', 'tp0=0', 'tp1=6', 'tsp=13', 'dsp=6', 'kvd=2', 'xop=O', 'iop=Q', 'tq0=34', 'tq1=35', 'inv0=32', 'inv1=34'))

import jax
import jax.numpy as jnp
import numpy as np
import jax.experimental.pallas as pl
import jax.experimental.pallas.tpu as pltpu

BF16 = jnp.bfloat16
F32 = jnp.float32
U32 = jnp.uint32

LANES = 128
LOG2E = 1.4426950408889634
CHUNK = 128


def _dft_tables():
    n = np.arange(CHUNK, dtype=np.float64)
    f = np.concatenate([np.arange(0, CHUNK, 2), np.arange(1, CHUNK, 2)]).astype(np.float64)
    theta = 2.0 * np.pi * (f[:, None] + 0.5) * n[None, :] / (2 * CHUNK)
    fwd = np.concatenate([np.cos(theta), -np.sin(theta)], axis=0)
    inv = np.concatenate([np.cos(theta).T, -np.sin(theta).T], axis=1) / CHUNK
    return fwd.astype(np.float32), inv.astype(np.float32)


_FWD, _INV = _dft_tables()


def _opt(name, default):
    for tok in DBG:
        if tok.startswith(name + "="):
            v = tok[len(name) + 1:]
            return int(v) if v.lstrip("-").isdigit() else v
    return default


def _mult(x, n):
    return x if isinstance(x, int) else pl.multiple_of(x, n)


def _rem(x, n):
    return x % n if isinstance(x, int) else jax.lax.rem(x, n)


NSLOT = 3


def _kernel(
    mem_hbm, shift_hbm, dvec_hbm, fwd_hbm, inv_hbm,
    x_hbm, wq_hbm, wk_hbm, wv_hbm, wo_hbm, bq_hbm, bk_hbm, bv_hbm, ssm_hbm,
    out_hbm,
    arena, wo, stage, xbuf, abuf, hbuf, accb,
    qb, kb, vb, sb, kf, xraw, xs, ks, ysf,
    mem_ref, shift_ref, dvec_ref, fwd_ref, inv_ref, sem_s, dvf,
    sem_w, sem_wo, sem_x, sem_q, sem_in, sem_ob, sem_a,
    *, S, DM, H, E, M, SEG, D, KS,
):
    L = M + SEG
    NSEG = S // SEG
    NCT = D // LANES
    NCH = S // CHUNK
    DCH = DM // NCT
    HP = H // 2
    NT = DM // LANES
    SPT = NSEG // NCT
    FPS = (CHUNK // 8) // SPT
    CPS = NCH // SPT
    XR = S // NCT
    TR = DM // 2
    SPEC = 2 * CHUNK
    NSP = NCH * SPEC // TR
    YS0 = 3 * H

    wq32 = wq_hbm.bitcast(U32)
    wk32 = wk_hbm.bitcast(U32)
    wv32 = wv_hbm.bitcast(U32)

    def lanes_of(c):
        return pl.ds(_mult(c * LANES, LANES), LANES)

    def b_in_copies(c):
        col = lanes_of(c)
        return (
            pltpu.make_async_copy(bk_hbm.at[:, col], kb.at[:, col], sem_in.at[c, 0]),
            pltpu.make_async_copy(bv_hbm.at[:, col], vb.at[:, col], sem_in.at[c, 1]),
            pltpu.make_async_copy(ssm_hbm.at[col, :], sb.at[col, :], sem_in.at[c, 2]),
        )

    def w_copies(c, slot):
        rows = pl.ds(_mult(c * DCH * HP, DCH * HP), DCH * HP)
        return tuple(
            pltpu.make_async_copy(w.at[rows, :], stage.at[slot, i], sem_w.at[slot, i])
            for i, w in enumerate((wq32, wk32, wv32))
        )

    WO32 = False

    def wo_copy(p):
        rows = pl.ds(_mult(p * (H * E // NCT), H * E // NCT), H * E // NCT)
        return pltpu.make_async_copy(wo_hbm.at[rows, :], wo.at[rows, :], sem_wo.at[p])

    def late_copies(c):
        rows = pl.ds(_mult(c * XR, XR), XR)
        return (
            pltpu.make_async_copy(x_hbm.at[rows, :], xbuf.at[rows, :], sem_x.at[c]),
            pltpu.make_async_copy(bq_hbm.at[:, lanes_of(c)], qb.at[:, lanes_of(c)], sem_q.at[c]),
        )

    def ob_copy(c, part):
        n = CPS * CHUNK
        rows = pl.ds(_mult(part * n, n), n)
        return pltpu.make_async_copy(qb.at[rows, lanes_of(c)], out_hbm.at[rows, lanes_of(NT + c)], sem_ob)

    def spec_rows(base, slot, j, r, n):
        tile = base + slot * NSP + j // (TR // SPEC)
        row = _mult((j % (TR // SPEC)) * SPEC + r, 8)
        return tile, pl.ds(row, n)

    def spec_load(base, slot, j, r, n):
        tile, rows = spec_rows(base, slot, j, r, n)
        return pltpu.bitcast(arena[tile, rows, :], F32)

    def spec_store(base, slot, j, r, val):
        tile, rows = spec_rows(base, slot, j, r, val.shape[0])
        arena[tile, rows, :] = pltpu.bitcast(val, U32)

    def relayout(c, slot, i):
        r0 = _mult(c * (DCH // 2), DCH // 2)

        def repack(words):
            return pltpu.bitcast(pltpu.bitcast(words, F32).astype(BF16), U32)

        if True:
            for j in range(HP):
                for dd in range(DCH // 16):
                    a = stage[slot, i, pl.ds(dd * 16 * HP + j, 8, stride=HP), :]
                    b = stage[slot, i, pl.ds((dd * 16 + 8) * HP + j, 8, stride=HP), :]
                    ab = jnp.concatenate([a, b], axis=0)
                    dst = pl.ds(r0 + dd * 8, 8)
                    arena[3 * (2 * j) + i, dst, :] = repack(ab << 16)
                    arena[3 * (2 * j + 1) + i, dst, :] = repack(ab & jnp.uint32(0xFFFF0000))

    def conv_taps(c):
        return shift_ref[:, lanes_of(c)].astype(F32)

    def stage_k(c, part):
        n = CPS * CHUNK
        kf[0:8, :] = jnp.where(part == 0, 0.0, kf[n:n + 8, :])
        kf[8:n + 8, :] = kb[pl.ds(_mult(part * n, n), n), lanes_of(c)].astype(F32)

    KVP = _opt("kvp", 4)

    def kv_piece(c, part, u, taps, piece):
        n = CHUNK // KVP
        j = part * CPS + u
        rows = pl.ds(_mult(j * CHUNK + piece * n, n), n)
        k0 = u * CHUNK + piece * n + 8
        acc = kf[k0:k0 + n, :] * taps[0:1, :]
        for t in range(1, KS):
            acc = acc + kf[k0 - t:k0 - t + n, :] * taps[t:t + 1, :]
        kv = (acc * vb[rows, lanes_of(c)].astype(F32)).astype(BF16)
        vb[rows, lanes_of(c)] = kv
        return kv

    def kv_chunk(c, part, u, taps):
        return jnp.concatenate([kv_piece(c, part, u, taps, q) for q in range(KVP)], axis=0)

    def x_spectrum(slot, part, u, kv):
        j = part * CPS + u
        half = CHUNK // 2
        xj = jnp.dot(fwd_ref[...], kv, preferred_element_type=F32)
        prev = xraw[u % 2]
        if u == 0:
            prev = jnp.where(part == 0, 0.0, prev)
        xraw[1 - u % 2] = xj
        xs[slot, j, 0:half, :] = xj[0:half] - prev[CHUNK:CHUNK + half]
        xs[slot, j, half:CHUNK, :] = xj[half:CHUNK] + prev[CHUNK + half:]
        xs[slot, j, CHUNK:CHUNK + half, :] = xj[CHUNK:CHUNK + half] + prev[0:half]
        xs[slot, j, CHUNK + half:, :] = xj[CHUNK + half:] - prev[half:CHUNK]

    def k_spectrum(c, slot, part, u):
        j = part * CPS + u
        blk = sb[lanes_of(c), pl.ds(_mult(j * CHUNK, CHUNK), CHUNK)]
        ks[slot, j] = jax.lax.dot_general(
            fwd_ref[...], blk, (((1,), (1,)), ((), ())), preferred_element_type=F32)

    GRP = _opt("grp", 2)

    def products(slot, fb, ig, free):
        r = _mult(fb * 8, 8)
        re, im = pl.ds(r, 8), pl.ds(r + CHUNK, 8)
        accs = [None] * GRP
        xv = {}
        for m in range(GRP * ig + GRP):
            kr = ks[slot, m, re, :]
            ki = ks[slot, m, im, :]
            for u in range(GRP):
                j = GRP * ig + u - m
                if j < 0:
                    continue
                if j not in xv:
                    xv[j] = (xs[slot, j, re, :], xs[slot, j, im, :])
                xr, xi = xv[j]
                if accs[u] is None:
                    accs[u] = (kr * xr - ki * xi, kr * xi + ki * xr)
                else:
                    ar, ai = accs[u]
                    accs[u] = (ar + kr * xr - ki * xi, ai + kr * xi + ki * xr)
            yield
        for u in range(GRP):
            if free:
                ysf[slot, GRP * ig + u, re, :] = accs[u][0]
                ysf[slot, GRP * ig + u, im, :] = accs[u][1]
            else:
                spec_store(YS0, slot, GRP * ig + u, r, accs[u][0])
                spec_store(YS0, slot, GRP * ig + u, r + CHUNK, accs[u][1])

    NFREE = _opt("nfree", 8)

    def is_free(f, ig):
        return f * (NCH // GRP) + ig >= NFREE

    def y_load(slot, i):
        pieces = []
        for blk in range(SPEC // 8):
            f = (blk % (CHUNK // 8)) % FPS
            pieces.append(lambda ig, blk=blk, f=f: None)
        return None

    def inverse(c, slot, i):
        cols = lanes_of(c)
        rows = pl.ds(_mult(i * CHUNK, CHUNK), CHUNK)
        dvec = dvf[pl.ds(c, 1), :]
        ya = spec_load(YS0, slot, i, 0, SPEC)
        yb = ysf[slot, i]
        pieces = []
        for blk in range(SPEC // 8):
            f = (blk % (CHUNK // 8)) % FPS
            rows8 = slice(blk * 8, blk * 8 + 8)
            nanch = sum(not is_free(f, ig) for ig in range(NCH // GRP))
            if nanch == 0:
                pieces.append(yb[rows8])
            elif nanch == NCH // GRP:
                pieces.append(ya[rows8])
            else:
                pieces.append(jnp.where(i < nanch * GRP, ya[rows8], yb[rows8]))
        yy = jnp.concatenate(pieces, axis=0)
        y = jnp.dot(inv_ref[...], yy.astype(BF16), preferred_element_type=F32)
        kv = vb[rows, cols].astype(F32)
        qv = qb[rows, cols].astype(F32)
        qb[rows, cols] = (qv * (y + kv * dvec)).astype(BF16)

    def spectra_part(c, slot, part, taps):
        stage_k(c, part)
        for u in range(CPS):
            x_spectrum(slot, part, u, kv_chunk(c, part, u, taps))
            k_spectrum(c, slot, part, u)

    small = [pltpu.make_async_copy(a, b, sem_s.at[i]) for i, (a, b) in enumerate(
        ((mem_hbm, mem_ref), (shift_hbm, shift_ref), (dvec_hbm, dvec_ref), (fwd_hbm, fwd_ref), (inv_hbm, inv_ref)))]
    for c0 in range(NSLOT - 1):
        for cp in w_copies(c0, c0):
            cp.start()
    for cp in small:
        cp.start()
    for c0 in range(2):
        for cp in b_in_copies(c0):
            cp.start()
    for cp in late_copies(0):
        cp.start()
    for cp in small:
        cp.wait()
    dvf[...] = dvec_ref[...].astype(F32)

    def pro_iter(c, carry):
        slot = jax.lax.rem(c, NSLOT)
        ahead = c + NSLOT - 1

        @pl.when(ahead < NCT)
        def _():
            for cp in w_copies(ahead, jax.lax.rem(ahead, NSLOT)):
                cp.start()

        WOA, WOB = _opt("woa", 1), _opt("wob", 3)
        for cc, lo, hi in ((NCT - 3, 0, WOA), (NCT - 2, WOA, WOB), (NCT - 1, WOB, NCT)):
            @pl.when(c == cc)
            def _(lo=lo, hi=hi):
                if lo == 0:
                    for cp in b_in_copies(2):
                        cp.start()
                for p in range(lo, hi):
                    wo_copy(p).start()
        for i, cp in enumerate(w_copies(c, slot)):
            cp.wait()
            if 'norelay' not in DBG:
                relayout(c, slot, i)

        @pl.when((c == 2) | (c == 3))
        def _():
            for cp in b_in_copies(c - 2):
                cp.wait()
            taps = conv_taps(c - 2)
            if 'nopro_sp' not in DBG:
                jax.lax.fori_loop(0, SPT, lambda part, z: (spectra_part(c - 2, c - 2, part, taps), z)[1], 0)

        @pl.when(c == 4)
        def _():
            def body(fb, z):
                for f in range(FPS):
                    for ig in range(NCH // GRP):
                        for _ in products(0, fb * FPS + f, ig, is_free(f, ig)):
                            pass
                return z
            if 'nopro_pr' not in DBG:
                jax.lax.fori_loop(0, CHUNK // 8 // FPS, body, 0)

        return carry

    jax.lax.fori_loop(0, NCT, pro_iter, 0)

    def start_late():
        for c0 in range(1, NCT):
            for cp in late_copies(c0):
                cp.start()
            if c0 >= 3:
                for cp in b_in_copies(c0):
                    cp.start()

    PEEL = 'nopeel' not in DBG
    if not PEEL:
        for p in range(NCT):
            wo_copy(p).wait()
        start_late()

    row = jax.lax.broadcasted_iota(jnp.int32, (L, L), 0)
    col = jax.lax.broadcasted_iota(jnp.int32, (L, L), 1)
    mask = (row < M) | (row >= col)
    scale = E ** -0.5
    hbuf[0:M, :] = mem_ref[...].astype(F32)
    ysf[2, 0, 0:8, :] = jnp.full((8, LANES), -1e9 / scale, F32)

    def wt(i):
        return pltpu.bitcast(arena[i], BF16)

    body_spec = [(w[0], int(w[1:])) for w in _opt("order", "K0_S1_Q0_P3_V1_O4").split("_")]
    maxlag = max(l for _, l in body_spec)
    ops = [(op, t - lag, t) for t in range(H + maxlag + 1) for op, lag in body_spec if 0 <= t - lag < H]

    def segment(s, carry, pos=0, first=False):
        _o = lambda name, d: _opt(name + '_' + 'abcd'[pos], _opt(name, d)) if not first else _opt(name, d)
        c = s // SPT
        part = s % SPT

        @pl.when(part == 0)
        def _():
            for cp in late_copies(c):
                cp.wait()

            @pl.when(c + 2 < NCT)
            def _():
                for cp in b_in_copies(c + 2):
                    cp.wait()

        c2 = _rem(c + 2, NCT)
        par = _rem(c, 2)

        nslots = len(ops)
        side = {}

        def at(n, fn):
            side.setdefault(min(n, nslots), []).append(fn)

        def slot_of(t, op="O"):
            for n, (o, hd, tt) in enumerate(ops):
                if tt > t or (tt == t and o == op):
                    return n
            return nslots

        if 'noB' not in DBG:
            st = {}
            n0 = slot_of(_o("tsp", 14))
            if 'nospec' not in DBG:
              at(n0, lambda: (stage_k(c2, part), st.update(taps=conv_taps(c2))))
            for u in range(0 if 'nospec' in DBG else CPS):
                nu = slot_of(_o("tsp", 14) + 1 + u * _o("dsp", 6))
                for q in range(KVP):
                    at(nu + q * _o("kvd", 1), lambda u=u, q=q: st.update({(u, q): kv_piece(c2, part, u, st["taps"], q)}))
                nx = slot_of(_o("tsp", 14) + 2 + u * _o("dsp", 6), _o("xop", "O"))
                at(nx, lambda u=u: x_spectrum(par, part, u, jnp.concatenate(
                    [st.pop((u, q)) for q in range(KVP)], axis=0)))
                at(nx + _o("dk", 0), lambda u=u: k_spectrum(c2, par, part, u))
            for u in range(0 if 'noinv' in DBG else CPS):
                at(slot_of(_o("inv%d" % u, 32 + 2 * u), _o("iop", "O")),
                   functools.partial(inverse, c, par, part * CPS + u))

            def prod_stream(free):
                for n in range(FPS * (NCH // GRP)):
                    f, ig = n // (NCH // GRP), n % (NCH // GRP)
                    if is_free(f, ig) == free:
                        yield from products(1 - par, part * FPS + f, ig, free)
                        yield

            for free, k0, k1 in ((False, "tp0", "tp1"), (True, "tq0", "tq1")):
                gen = prod_stream(free)
                nmicro = sum(GRP * ig + GRP + 1 for f in range(FPS) for ig in range(NCH // GRP)
                             if is_free(f, ig) == free)
                p0 = slot_of(_o(k0, 30 if free else 0))
                p1 = slot_of(_o(k1, 31 if free else 13))
                for n in range(0 if 'noprod' in DBG else nmicro):
                    at(p0 + n * (p1 - p0) // nmicro, lambda gen=gen: next(gen))

        r0 = _mult(s * SEG, SEG)
        hbuf[M:L, :] = xbuf[pl.ds(r0, SEG), :].astype(F32)
        h = hbuf[...]
        if 'pin' in DBG:
            neg = ysf[2 + _mult(s // NSEG, 1), 0, 0:1, 0:L]
        else:
            neg = -1e9 / scale
        Q, K, V, P, O, Z = {}, {}, {}, {}, {}, {}
        acc = [None] * NT

        for n, (op, hd, t) in enumerate(ops):
            for fn in side.pop(n, []):
                fn()
            if op == "Q":
                Q[hd] = jnp.dot(h, wt(3 * hd), preferred_element_type=F32)
            elif op == "K":
                K[hd] = jnp.dot(h, wt(3 * hd + 1), preferred_element_type=F32).astype(BF16)
            elif op == "V":
                V[hd] = jnp.dot(h, wt(3 * hd + 2), preferred_element_type=F32).astype(BF16)
            elif op == "S":
                sc = jax.lax.dot_general(Q.pop(hd), K.pop(hd), (((1,), (1,)), ((), ())),
                                         preferred_element_type=F32)
                sc = jnp.where(mask, sc, neg)
                p = jnp.exp2((sc - jnp.max(sc, axis=-1, keepdims=True)) * (scale * LOG2E))
                P[hd] = p
                Z[hd] = jnp.sum(p, axis=-1, keepdims=True)
            elif op == "P":
                z = Z.pop(hd)
                r = pltpu.reciprocal(z, approx=True)
                r = r * (2.0 - z * r)
                O[hd] = jnp.dot(P.pop(hd), V.pop(hd), preferred_element_type=F32) * r
            elif op == "O":
                if first and hd % (H // NCT) == 0:
                    wo_copy(hd // (H // NCT)).wait()
                    if hd == H - H // NCT:
                        start_late()
                o = O.pop(hd)
                for n in range(NT):
                    if WO32:
                        w = pltpu.bitcast(wo[n, hd * (E // 2):(hd + 1) * (E // 2), :], BF16)
                    else:
                        w = wo[hd * E:(hd + 1) * E, n * LANES:(n + 1) * LANES]
                    y = jnp.dot(o, w, preferred_element_type=F32)
                    if 'accreg' in DBG:
                        acc[n] = y if acc[n] is None else acc[n] + y
                    elif hd == 0:
                        accb[:, n * LANES:(n + 1) * LANES] = y
                    elif hd < H - 1:
                        accb[:, n * LANES:(n + 1) * LANES] += y
                    else:
                        acc[n] = accb[:, n * LANES:(n + 1) * LANES] + y
        for t in sorted(side):
            for fn in side[t]:
                fn()
        out = jnp.concatenate(acc, axis=1).astype(BF16)
        hbuf[0:M, :] = out[0:M].astype(F32)
        abuf[pl.ds(r0, SEG), :] = out[M:L]
        pltpu.make_async_copy(
            abuf.at[pl.ds(r0, SEG), :], out_hbm.at[pl.ds(r0, SEG), pl.ds(0, DM)], sem_a
        ).start()
        ob_copy(c, part).start()
        return carry

    nst = _opt("steps", NSEG)
    UNR = _opt("unr", 1)

    s0 = 0
    if PEEL and nst > 0:
        segment(0, 0, 0, first=True)
        s0 = 1
        while (nst - s0) % UNR:
            segment(s0, 0, 0)
            s0 += 1
    elif PEEL:
        for p in range(NCT):
            wo_copy(p).wait()
        start_late()

    def steps(i, carry):
        for u in range(UNR):
            segment(s0 + i * UNR + u, carry, u)
        return carry

    if 'dyn' in DBG:
        zero = (dvec_ref[0:1, :].astype(F32) * 0.0).astype(jnp.int32)
        jax.lax.fori_loop(0, (nst - s0) // UNR + jnp.max(zero), steps, 0)
    else:
        jax.lax.fori_loop(0, (nst - s0) // UNR, steps, 0)

    if 'keep' in DBG:
        z0 = jnp.max((dvec_ref[0:1, :].astype(F32) * 0.0).astype(jnp.int32))
        hbuf[0:8, 0:128] = xs[z0, z0, 0:8, :] + ks[z0, z0, 0:8, :] + spec_load(YS0, z0, z0, 0, 8)
        abuf[0:8, 0:128] = hbuf[0:8, 0:128].astype(BF16)
    if nst == NSEG:
        pltpu.make_async_copy(qb, qb, sem_ob).wait()
        pltpu.make_async_copy(abuf, out_hbm.at[:, pl.ds(0, DM)], sem_a).wait()
    else:
        nblk = -(-nst // SPT)
        for cc in range(nblk, NCT):
            for cp in late_copies(cc):
                cp.wait()
        for cc in range(max(nblk + 2, 2), NCT):
            for cp in b_in_copies(cc):
                cp.wait()
        for ss in range(nst):
            ob_copy(ss // SPT, ss % SPT).wait()
        if nst:
            pltpu.make_async_copy(abuf.at[0:nst * SEG], out_hbm.at[0:nst * SEG, pl.ds(0, DM)], sem_a).wait()


@functools.partial(jax.jit, static_argnames=("A_seg_len",))
def pallas_concat_heads__memory_aug_recurrent_mem_tr__ssm_conv_h3__prompt_kernel(
    A_x: jax.Array,
    A_mem0: jax.Array,
    A_Wq: jax.Array,
    A_Wk: jax.Array,
    A_Wv: jax.Array,
    A_Wo: jax.Array,
    A_seg_len: int,
    B_q: jax.Array,
    B_k: jax.Array,
    B_v: jax.Array,
    B_shift_k: jax.Array,
    B_ssm_k: jax.Array,
    B_ssm_D: jax.Array,
):
    B, S, DM = A_x.shape
    H, E = A_Wq.shape[1], A_Wq.shape[2]
    M = A_mem0.shape[1]
    SEG = int(A_seg_len)
    D = B_q.shape[2]
    KS = B_shift_k.shape[1]
    assert B == 1 and E == LANES and S % CHUNK == 0 and S % SEG == 0
    NCT = D // LANES
    NCH = S // CHUNK
    DCH = DM // NCT
    NSP = NCH * 2 * CHUNK // (DM // 2)
    CPS = NCH // (S // SEG // NCT)

    kernel = functools.partial(_kernel, S=S, DM=DM, H=H, E=E, M=M, SEG=SEG, D=D, KS=KS)
    vmem = pl.BlockSpec(memory_space=pltpu.VMEM)
    hbm = pl.BlockSpec(memory_space=pl.ANY)
    dma = pltpu.SemaphoreType.DMA

    out = pl.pallas_call(
        kernel,
        out_shape=jax.ShapeDtypeStruct((S, DM + D), BF16),
        in_specs=[hbm] * 14,
        out_specs=hbm,
        scratch_shapes=[
            pltpu.VMEM((3 * H + 2 * NSP, DM // 2, E), U32),
            pltpu.VMEM((H * E, DM), BF16) if True else pltpu.VMEM((DM // LANES, H * E // 2, LANES), U32),
            pltpu.VMEM((NSLOT, 3, DCH * (H // 2), E), U32),
            pltpu.VMEM((S, DM), BF16),
            pltpu.VMEM((S, DM), BF16),
            pltpu.VMEM((M + SEG, DM), F32),
            pltpu.VMEM((M + SEG, DM), F32),
            pltpu.VMEM((S, D), BF16),
            pltpu.VMEM((S, D), BF16),
            pltpu.VMEM((S, D), BF16),
            pltpu.VMEM((D, S), BF16),
            pltpu.VMEM((8 + CPS * CHUNK, LANES), F32),
            pltpu.VMEM((2, 2 * CHUNK, LANES), F32),
            pltpu.VMEM((2, NCH, 2 * CHUNK, LANES), F32),
            pltpu.VMEM((2, NCH, 2 * CHUNK, LANES), F32),
            pltpu.VMEM((3, NCH, 2 * CHUNK, LANES), F32),
            pltpu.VMEM((M, DM), BF16), pltpu.VMEM((KS, D), BF16), pltpu.VMEM((NCT, LANES), BF16),
            pltpu.VMEM((2 * CHUNK, CHUNK), BF16), pltpu.VMEM((CHUNK, 2 * CHUNK), BF16), dma((5,)),
            pltpu.VMEM((NCT, LANES), F32),
            dma((NSLOT, 3)), dma((NCT,)), dma((NCT,)), dma((NCT,)), dma((NCT, 3)), dma, dma,
        ],
        compiler_params=pltpu.CompilerParams(vmem_limit_bytes=124 * 1024 * 1024),
    )(
        A_mem0.reshape(M, DM), B_shift_k.T, B_ssm_D.reshape(NCT, LANES),
        jnp.asarray(_FWD, BF16), jnp.asarray(_INV, BF16),
        A_x.reshape(S, DM),
        A_Wq.reshape(DM * H, E), A_Wk.reshape(DM * H, E), A_Wv.reshape(DM * H, E),
        A_Wo.reshape(H * E, DM),
        B_q.reshape(S, D), B_k.reshape(S, D), B_v.reshape(S, D), B_ssm_k,
    )
    return out.reshape(B, S, DM + D)
```

```python
import functools


DBG = frozenset(('order=K0_P3_Q0_S1_V1_O4', 'grp=2', 'nfree=10', 'tp0=2', 'tp1=8', 'tsp=13', 'dsp=6', 'kvd=1', 'xop=K', 'iop=Q', 'tq0=28', 'tq1=29', 'inv0=32', 'inv1=34', 'dk=1', 'kvp=4'))

import jax
import jax.numpy as jnp
import numpy as np
import jax.experimental.pallas as pl
import jax.experimental.pallas.tpu as pltpu

BF16 = jnp.bfloat16
F32 = jnp.float32
U32 = jnp.uint32

LANES = 128
LOG2E = 1.4426950408889634
CHUNK = 128


def _dft_tables():
    n = np.arange(CHUNK, dtype=np.float64)
    f = np.concatenate([np.arange(0, CHUNK, 2), np.arange(1, CHUNK, 2)]).astype(np.float64)
    theta = 2.0 * np.pi * (f[:, None] + 0.5) * n[None, :] / (2 * CHUNK)
    fwd = np.concatenate([np.cos(theta), -np.sin(theta)], axis=0)
    inv = np.concatenate([np.cos(theta).T, -np.sin(theta).T], axis=1) / CHUNK
    return fwd.astype(np.float32), inv.astype(np.float32)


_FWD, _INV = _dft_tables()


def _opt(name, default):
    for tok in DBG:
        if tok.startswith(name + "="):
            v = tok[len(name) + 1:]
            return int(v) if v.lstrip("-").isdigit() else v
    return default


def _mult(x, n):
    return x if isinstance(x, int) else pl.multiple_of(x, n)


def _rem(x, n):
    return x % n if isinstance(x, int) else jax.lax.rem(x, n)


NSLOT = 3


def _kernel(
    mem_hbm, shift_hbm, dvec_hbm, fwd_hbm, inv_hbm,
    x_hbm, wq_hbm, wk_hbm, wv_hbm, wo_hbm, bq_hbm, bk_hbm, bv_hbm, ssm_hbm,
    out_hbm,
    arena, wo, stage, xbuf, abuf, hbuf, accb,
    qb, kb, vb, sb, kf, xraw, xs, ks, ysf,
    mem_ref, shift_ref, dvec_ref, fwd_ref, inv_ref, sem_s, dvf,
    sem_w, sem_wo, sem_x, sem_q, sem_in, sem_ob, sem_a,
    *, S, DM, H, E, M, SEG, D, KS,
):
    L = M + SEG
    NSEG = S // SEG
    NCT = D // LANES
    NCH = S // CHUNK
    DCH = DM // NCT
    HP = H // 2
    NT = DM // LANES
    SPT = NSEG // NCT
    FPS = (CHUNK // 8) // SPT
    CPS = NCH // SPT
    XR = S // NCT
    EARLY = _opt('early', 2)
    TR = DM // 2
    SPEC = 2 * CHUNK
    NSP = NCH * SPEC // TR
    YS0 = 3 * H

    wq32 = wq_hbm.bitcast(U32)
    wk32 = wk_hbm.bitcast(U32)
    wv32 = wv_hbm.bitcast(U32)

    def lanes_of(c):
        return pl.ds(_mult(c * LANES, LANES), LANES)

    def b_in_copies(c, part=None):
        col = lanes_of(c)
        if part is None:
            t, sem = slice(None), sem_in.at[c]
        else:
            t = slice(0, EARLY * CPS * CHUNK) if part == 0 else slice(EARLY * CPS * CHUNK, S)
            sem = sem_in.at[NCT + part]
        return (
            pltpu.make_async_copy(bk_hbm.at[t, col], kb.at[t, col], sem.at[0]),
            pltpu.make_async_copy(bv_hbm.at[t, col], vb.at[t, col], sem.at[1]),
            pltpu.make_async_copy(ssm_hbm.at[col, t], sb.at[col, t], sem.at[2]),
        )

    def w_copies(c, slot):
        rows = pl.ds(_mult(c * DCH * HP, DCH * HP), DCH * HP)
        return tuple(
            pltpu.make_async_copy(w.at[rows, :], stage.at[slot, i], sem_w.at[slot, i])
            for i, w in enumerate((wq32, wk32, wv32))
        )

    WO32 = False

    def wo_copy(p):
        rows = pl.ds(_mult(p * (H * E // NCT), H * E // NCT), H * E // NCT)
        return pltpu.make_async_copy(wo_hbm.at[rows, :], wo.at[rows, :], sem_wo.at[p])

    def late_copies(c, part=None):
        if part is None:
            rows, t, sc = pl.ds(_mult(c * XR, XR), XR), slice(None), c
        else:
            rows = slice(0, EARLY * SEG) if part == 0 else slice(EARLY * SEG, XR)
            t = slice(0, EARLY * CPS * CHUNK) if part == 0 else slice(EARLY * CPS * CHUNK, S)
            sc = NCT + part
        return (
            pltpu.make_async_copy(x_hbm.at[rows, :], xbuf.at[rows, :], sem_x.at[sc]),
            pltpu.make_async_copy(bq_hbm.at[t, lanes_of(c)], qb.at[t, lanes_of(c)], sem_q.at[sc]),
        )

    def first_block_copies(part):
        return late_copies(0, part) + b_in_copies(2, part)

    def ob_copy(c, part):
        n = CPS * CHUNK
        rows = pl.ds(_mult(part * n, n), n)
        return pltpu.make_async_copy(qb.at[rows, lanes_of(c)], out_hbm.at[rows, lanes_of(NT + c)], sem_ob)

    def spec_rows(base, slot, j, r, n):
        tile = base + slot * NSP + j // (TR // SPEC)
        row = _mult((j % (TR // SPEC)) * SPEC + r, 8)
        return tile, pl.ds(row, n)

    def spec_load(base, slot, j, r, n):
        tile, rows = spec_rows(base, slot, j, r, n)
        return pltpu.bitcast(arena[tile, rows, :], F32)

    def spec_store(base, slot, j, r, val):
        tile, rows = spec_rows(base, slot, j, r, val.shape[0])
        arena[tile, rows, :] = pltpu.bitcast(val, U32)

    def relayout(c, slot, i):
        r0 = _mult(c * (DCH // 2), DCH // 2)

        def repack(words):
            return pltpu.bitcast(pltpu.bitcast(words, F32).astype(BF16), U32)

        if True:
            for j in range(HP):
                for dd in range(DCH // 16):
                    a = stage[slot, i, pl.ds(dd * 16 * HP + j, 8, stride=HP), :]
                    b = stage[slot, i, pl.ds((dd * 16 + 8) * HP + j, 8, stride=HP), :]
                    ab = jnp.concatenate([a, b], axis=0)
                    dst = pl.ds(r0 + dd * 8, 8)
                    arena[3 * (2 * j) + i, dst, :] = repack(ab << 16)
                    arena[3 * (2 * j + 1) + i, dst, :] = repack(ab & jnp.uint32(0xFFFF0000))

    def conv_taps(c):
        return shift_ref[:, lanes_of(c)].astype(F32)

    def stage_k(c, part):
        n = CPS * CHUNK
        kf[0:8, :] = jnp.where(part == 0, 0.0, kf[n:n + 8, :])
        kf[8:n + 8, :] = kb[pl.ds(_mult(part * n, n), n), lanes_of(c)].astype(F32)

    KVP = _opt("kvp", 4)

    def kv_piece(c, part, u, taps, piece):
        n = CHUNK // KVP
        j = part * CPS + u
        rows = pl.ds(_mult(j * CHUNK + piece * n, n), n)
        k0 = u * CHUNK + piece * n + 8
        acc = kf[k0:k0 + n, :] * taps[0:1, :]
        for t in range(1, KS):
            acc = acc + kf[k0 - t:k0 - t + n, :] * taps[t:t + 1, :]
        kv = (acc * vb[rows, lanes_of(c)].astype(F32)).astype(BF16)
        vb[rows, lanes_of(c)] = kv
        return kv

    def kv_chunk(c, part, u, taps):
        return jnp.concatenate([kv_piece(c, part, u, taps, q) for q in range(KVP)], axis=0)

    def x_spectrum(slot, part, u, kv):
        j = part * CPS + u
        half = CHUNK // 2
        xj = jnp.dot(fwd_ref[...], kv, preferred_element_type=F32)
        prev = xraw[u % 2]
        if u == 0:
            prev = jnp.where(part == 0, 0.0, prev)
        xraw[1 - u % 2] = xj
        xs[slot, j, 0:half, :] = xj[0:half] - prev[CHUNK:CHUNK + half]
        xs[slot, j, half:CHUNK, :] = xj[half:CHUNK] + prev[CHUNK + half:]
        xs[slot, j, CHUNK:CHUNK + half, :] = xj[CHUNK:CHUNK + half] + prev[0:half]
        xs[slot, j, CHUNK + half:, :] = xj[CHUNK + half:] - prev[half:CHUNK]

    def k_spectrum(c, slot, part, u):
        j = part * CPS + u
        blk = sb[lanes_of(c), pl.ds(_mult(j * CHUNK, CHUNK), CHUNK)]
        ks[slot, j] = jax.lax.dot_general(
            fwd_ref[...], blk, (((1,), (1,)), ((), ())), preferred_element_type=F32)

    GRP = _opt("grp", 2)

    def products(slot, fb, ig, free):
        r = _mult(fb * 8, 8)
        re, im = pl.ds(r, 8), pl.ds(r + CHUNK, 8)
        accs = [None] * GRP
        xv = {}
        for m in range(GRP * ig + GRP):
            kr = ks[slot, m, re, :]
            ki = ks[slot, m, im, :]
            for u in range(GRP):
                j = GRP * ig + u - m
                if j < 0:
                    continue
                if j not in xv:
                    xv[j] = (xs[slot, j, re, :], xs[slot, j, im, :])
                xr, xi = xv[j]
                if accs[u] is None:
                    accs[u] = (kr * xr - ki * xi, kr * xi + ki * xr)
                else:
                    ar, ai = accs[u]
                    accs[u] = (ar + kr * xr - ki * xi, ai + kr * xi + ki * xr)
            yield
        for u in range(GRP):
            if free:
                ysf[slot, GRP * ig + u, re, :] = accs[u][0]
                ysf[slot, GRP * ig + u, im, :] = accs[u][1]
            else:
                spec_store(YS0, slot, GRP * ig + u, r, accs[u][0])
                spec_store(YS0, slot, GRP * ig + u, r + CHUNK, accs[u][1])

    NFREE = _opt("nfree", 8)

    def is_free(f, ig):
        return f * (NCH // GRP) + ig >= NFREE

    def y_load(slot, i):
        pieces = []
        for blk in range(SPEC // 8):
            f = (blk % (CHUNK // 8)) % FPS
            pieces.append(lambda ig, blk=blk, f=f: None)
        return None

    def inverse(c, slot, i):
        cols = lanes_of(c)
        rows = pl.ds(_mult(i * CHUNK, CHUNK), CHUNK)
        dvec = dvf[pl.ds(c, 1), :]
        ya = spec_load(YS0, slot, i, 0, SPEC)
        yb = ysf[slot, i]
        pieces = []
        for blk in range(SPEC // 8):
            f = (blk % (CHUNK // 8)) % FPS
            rows8 = slice(blk * 8, blk * 8 + 8)
            nanch = sum(not is_free(f, ig) for ig in range(NCH // GRP))
            if nanch == 0:
                pieces.append(yb[rows8])
            elif nanch == NCH // GRP:
                pieces.append(ya[rows8])
            else:
                pieces.append(jnp.where(i < nanch * GRP, ya[rows8], yb[rows8]))
        yy = jnp.concatenate(pieces, axis=0)
        y = jnp.dot(inv_ref[...], yy.astype(BF16), preferred_element_type=F32)
        kv = vb[rows, cols].astype(F32)
        qv = qb[rows, cols].astype(F32)
        qb[rows, cols] = (qv * (y + kv * dvec)).astype(BF16)

    def spectra_part(c, slot, part, taps):
        stage_k(c, part)
        for u in range(CPS):
            x_spectrum(slot, part, u, kv_chunk(c, part, u, taps))
            k_spectrum(c, slot, part, u)

    small = [pltpu.make_async_copy(a, b, sem_s.at[i]) for i, (a, b) in enumerate(
        ((mem_hbm, mem_ref), (shift_hbm, shift_ref), (dvec_hbm, dvec_ref), (fwd_hbm, fwd_ref), (inv_hbm, inv_ref)))]
    for c0 in range(NSLOT - 1):
        for cp in w_copies(c0, c0):
            cp.start()
    for cp in small:
        cp.start()
    for c0 in range(2):
        for cp in b_in_copies(c0):
            cp.start()
    for cp in first_block_copies(0):
        cp.start()
    for cp in small:
        cp.wait()
    dvf[...] = dvec_ref[...].astype(F32)

    WOD = _opt("wod", 3)

    def pro_iter(c, carry):
        slot = jax.lax.rem(c, NSLOT)
        ahead = c + NSLOT - 1

        @pl.when(ahead < NCT)
        def _():
            for cp in w_copies(ahead, jax.lax.rem(ahead, NSLOT)):
                cp.start()

        WOA, WOB = _opt("woa", 1), _opt("wob", 3)
        for cc, lo, hi in ((NCT - 3, 0, WOA), (NCT - 2, WOA, WOB), (NCT - 1, WOB, WOD)):
            @pl.when(c == cc)
            def _(lo=lo, hi=hi):
                for p in range(lo, hi):
                    wo_copy(p).start()
        for i, cp in enumerate(w_copies(c, slot)):
            cp.wait()
            if 'norelay' not in DBG:
                relayout(c, slot, i)

        @pl.when((c == 2) | (c == 3))
        def _():
            for cp in b_in_copies(c - 2):
                cp.wait()
            taps = conv_taps(c - 2)
            if 'nopro_sp' not in DBG:
                jax.lax.fori_loop(0, SPT, lambda part, z: (spectra_part(c - 2, c - 2, part, taps), z)[1], 0)

        @pl.when(c == 4)
        def _():
            def body(fb, z):
                for f in range(FPS):
                    for ig in range(NCH // GRP):
                        for _ in products(0, fb * FPS + f, ig, is_free(f, ig)):
                            pass
                return z
            if 'nopro_pr' not in DBG:
                jax.lax.fori_loop(0, CHUNK // 8 // FPS, body, 0)

        return carry

    jax.lax.fori_loop(0, NCT, pro_iter, 0)

    def start_late():
        for c0 in range(1, 1 if 'nolate' in DBG else NCT):
            for cp in late_copies(c0):
                cp.start()
            if c0 >= 3:
                for cp in b_in_copies(c0):
                    cp.start()

    PEEL = 'nopeel' not in DBG
    if not PEEL:
        for p in range(WOD, NCT):
            wo_copy(p).start()
        for p in range(NCT):
            wo_copy(p).wait()
        for cp in first_block_copies(1):
            cp.start()
            cp.wait()
        start_late()

    row = jax.lax.broadcasted_iota(jnp.int32, (L, L), 0)
    col = jax.lax.broadcasted_iota(jnp.int32, (L, L), 1)
    mask = (row < M) | (row >= col)
    scale = E ** -0.5
    hbuf[0:M, :] = mem_ref[...].astype(F32)
    ysf[2, 0, 0:8, :] = jnp.full((8, LANES), -1e9 / scale, F32)

    def wt(i):
        return pltpu.bitcast(arena[i], BF16)

    body_spec = [(w[0], int(w[1:])) for w in _opt("order", "K0_S1_Q0_P3_V1_O4").split("_")]
    maxlag = max(l for _, l in body_spec)
    ops = [(op, t - lag, t) for t in range(H + maxlag + 1) for op, lag in body_spec if 0 <= t - lag < H]

    def wait_block_inputs(c):
        for cp in late_copies(c):
            cp.wait()

        @pl.when(c + 2 < NCT)
        def _():
            for cp in b_in_copies(c + 2):
                cp.wait()

    def send_outputs(s, n):
        rows = pl.ds(_mult(s * SEG, SEG), n * SEG)
        pltpu.make_async_copy(abuf.at[rows, :], out_hbm.at[rows, pl.ds(0, DM)], sem_a).start()
        for u in range(n):
            ob_copy((s + u) // SPT, (s + u) % SPT).start()

    def segment(s, carry, pos=0, first=False):
        _o = lambda name, d: _opt(name + '_' + 'abcd'[pos], _opt(name, d)) if not first else _opt(name, d)
        c = s // SPT
        part = s % SPT

        c2 = _rem(c + 2, NCT)
        par = _rem(c, 2)

        nslots = len(ops)
        side = {}

        def at(n, fn):
            side.setdefault(min(n, nslots), []).append(fn)

        def slot_of(t, op="O"):
            for n, (o, hd, tt) in enumerate(ops):
                if tt > t or (tt == t and o == op):
                    return n
            return nslots

        if 'noB' not in DBG:
            st = {}
            n0 = slot_of(_o("tsp", 14))
            if 'nospec' not in DBG:
              at(n0, lambda: (stage_k(c2, part), st.update(taps=conv_taps(c2))))
            for u in range(0 if 'nospec' in DBG else CPS):
                nu = slot_of(_o("tsp", 14) + 1 + u * _o("dsp", 6))
                for q in range(KVP):
                    at(nu + q * _o("kvd", 1), lambda u=u, q=q: st.update({(u, q): kv_piece(c2, part, u, st["taps"], q)}))
                nx = max(slot_of(_o("tsp", 14) + 2 + u * _o("dsp", 6), _o("xop", "O")),
                         nu + (KVP - 1) * _o("kvd", 1))
                at(nx, lambda u=u: x_spectrum(par, part, u, jnp.concatenate(
                    [st.pop((u, q)) for q in range(KVP)], axis=0)))
                at(nx + _o("dk", 0), lambda u=u: k_spectrum(c2, par, part, u))
            for u in range(0 if 'noinv' in DBG else CPS):
                at(slot_of(_o("inv%d" % u, 32 + 2 * u), _o("iop", "O")),
                   functools.partial(inverse, c, par, part * CPS + u))

            def prod_stream(free):
                for n in range(FPS * (NCH // GRP)):
                    f, ig = n // (NCH // GRP), n % (NCH // GRP)
                    if is_free(f, ig) == free:
                        yield from products(1 - par, part * FPS + f, ig, free)
                        yield

            for free, k0, k1 in ((False, "tp0", "tp1"), (True, "tq0", "tq1")):
                gen = prod_stream(free)
                nmicro = sum(GRP * ig + GRP + 1 for f in range(FPS) for ig in range(NCH // GRP)
                             if is_free(f, ig) == free)
                p0 = slot_of(_o(k0, 30 if free else 0))
                p1 = slot_of(_o(k1, 31 if free else 13))
                for n in range(0 if 'noprod' in DBG else nmicro):
                    at(p0 + n * (p1 - p0) // nmicro, lambda gen=gen: next(gen))

        r0 = _mult(s * SEG, SEG)
        hbuf[M:L, :] = xbuf[pl.ds(r0, SEG), :].astype(F32)
        h = hbuf[...]
        if 'pin' in DBG:
            neg = ysf[2 + _mult(s // NSEG, 1), 0, 0:1, 0:L]
        else:
            neg = -1e9 / scale
        Q, K, V, P, O, Z = {}, {}, {}, {}, {}, {}
        acc = [None] * NT

        for n, (op, hd, t) in enumerate(ops):
            for fn in side.pop(n, []):
                fn()
            if op == "Q":
                Q[hd] = jnp.dot(h, wt(3 * hd), preferred_element_type=F32)
            elif op == "K":
                K[hd] = jnp.dot(h, wt(3 * hd + 1), preferred_element_type=F32).astype(BF16)
            elif op == "V":
                V[hd] = jnp.dot(h, wt(3 * hd + 2), preferred_element_type=F32).astype(BF16)
            elif op == "S":
                sc = jax.lax.dot_general(Q.pop(hd), K.pop(hd), (((1,), (1,)), ((), ())),
                                         preferred_element_type=F32)
                sc = jnp.where(mask, sc, neg)
                p = jnp.exp2((sc - jnp.max(sc, axis=-1, keepdims=True)) * (scale * LOG2E))
                P[hd] = p
                Z[hd] = jnp.sum(p, axis=-1, keepdims=True)
            elif op == "P":
                z = Z.pop(hd)
                r = pltpu.reciprocal(z, approx=True)
                r = r * (2.0 - z * r)
                O[hd] = jnp.dot(P.pop(hd), V.pop(hd), preferred_element_type=F32) * r
            elif op == "O":
                if first and hd % (H // NCT) == 0:
                    wo_copy(hd // (H // NCT)).wait()
                    if hd // (H // NCT) + WOD < NCT:
                        wo_copy(hd // (H // NCT) + WOD).start()
                    if hd == H - _opt('fb1', 1) * H // NCT:
                        for cp in first_block_copies(1):
                            cp.start()
                o = O.pop(hd)
                for n in range(NT):
                    if WO32:
                        w = pltpu.bitcast(wo[n, hd * (E // 2):(hd + 1) * (E // 2), :], BF16)
                    else:
                        w = wo[hd * E:(hd + 1) * E, n * LANES:(n + 1) * LANES]
                    y = jnp.dot(o, w, preferred_element_type=F32)
                    if 'accreg' in DBG:
                        acc[n] = y if acc[n] is None else acc[n] + y
                    elif hd == 0:
                        accb[:, n * LANES:(n + 1) * LANES] = y
                    elif hd < H - 1:
                        accb[:, n * LANES:(n + 1) * LANES] += y
                    else:
                        acc[n] = accb[:, n * LANES:(n + 1) * LANES] + y
        for t in sorted(side):
            for fn in side[t]:
                fn()
        out = jnp.concatenate(acc, axis=1).astype(BF16)
        hbuf[0:M, :] = out[0:M].astype(F32)
        abuf[pl.ds(r0, SEG), :] = out[M:L]
        send_outputs(s, 1)
        nxt = s + 1

        @pl.when((nxt % SPT == 0) & (nxt < NSEG))
        def _():
            wait_block_inputs(nxt // SPT)

        return carry

    nst = _opt("steps", NSEG)
    UNR = _opt("unr", 1)

    assert UNR == 1 and PEEL
    s0 = 0
    if nst > 0:
        for cp in first_block_copies(0):
            cp.wait()
        segment(0, 0, 0, first=True)
        s0 = 1
        while s0 < min(EARLY, nst):
            segment(s0, 0, 0)
            s0 += 1
        for cp in first_block_copies(1):
            cp.wait()
        start_late()
    else:
        for cp in first_block_copies(0):
            cp.wait()
        for p in range(WOD, NCT):
            wo_copy(p).start()
        for p in range(NCT):
            wo_copy(p).wait()
        for cp in first_block_copies(1):
            cp.start()
            cp.wait()
        start_late()

    def steps(i, carry):
        segment(s0 + i, carry, 0)
        return carry

    if 'dyn' in DBG:
        zero = (dvec_ref[0:1, :].astype(F32) * 0.0).astype(jnp.int32)
        jax.lax.fori_loop(0, (nst - s0) // UNR + jnp.max(zero), steps, 0)
    else:
        jax.lax.fori_loop(0, (nst - s0) // UNR, steps, 0)

    if 'keep' in DBG:
        z0 = jnp.max((dvec_ref[0:1, :].astype(F32) * 0.0).astype(jnp.int32))
        hbuf[0:8, 0:128] = xs[z0, z0, 0:8, :] + ks[z0, z0, 0:8, :] + spec_load(YS0, z0, z0, 0, 8)
        abuf[0:8, 0:128] = hbuf[0:8, 0:128].astype(BF16)
    if nst == NSEG:
        pltpu.make_async_copy(qb, qb, sem_ob).wait()
        pltpu.make_async_copy(abuf, out_hbm.at[:, pl.ds(0, DM)], sem_a).wait()
    else:
        nblk = nst // SPT + 1 if nst else 0
        for cc in range(max(nblk, 1), 1 if 'nolate' in DBG else NCT):
            for cp in late_copies(cc):
                cp.wait()
        for cc in range(max(nblk + 2, 3), 3 if 'nolate' in DBG else NCT):
            for cp in b_in_copies(cc):
                cp.wait()
        for ss in range(nst):
            ob_copy(ss // SPT, ss % SPT).wait()
        if nst:
            pltpu.make_async_copy(abuf.at[0:nst * SEG], out_hbm.at[0:nst * SEG, pl.ds(0, DM)], sem_a).wait()


@functools.partial(jax.jit, static_argnames=("A_seg_len",))
def pallas_concat_heads__memory_aug_recurrent_mem_tr__ssm_conv_h3__prompt_kernel(
    A_x: jax.Array,
    A_mem0: jax.Array,
    A_Wq: jax.Array,
    A_Wk: jax.Array,
    A_Wv: jax.Array,
    A_Wo: jax.Array,
    A_seg_len: int,
    B_q: jax.Array,
    B_k: jax.Array,
    B_v: jax.Array,
    B_shift_k: jax.Array,
    B_ssm_k: jax.Array,
    B_ssm_D: jax.Array,
):
    B, S, DM = A_x.shape
    H, E = A_Wq.shape[1], A_Wq.shape[2]
    M = A_mem0.shape[1]
    SEG = int(A_seg_len)
    D = B_q.shape[2]
    KS = B_shift_k.shape[1]
    assert B == 1 and E == LANES and S % CHUNK == 0 and S % SEG == 0
    NCT = D // LANES
    NCH = S // CHUNK
    DCH = DM // NCT
    NSP = NCH * 2 * CHUNK // (DM // 2)
    CPS = NCH // (S // SEG // NCT)

    kernel = functools.partial(_kernel, S=S, DM=DM, H=H, E=E, M=M, SEG=SEG, D=D, KS=KS)
    vmem = pl.BlockSpec(memory_space=pltpu.VMEM)
    hbm = pl.BlockSpec(memory_space=pl.ANY)
    dma = pltpu.SemaphoreType.DMA

    out = pl.pallas_call(
        kernel,
        out_shape=jax.ShapeDtypeStruct((S, DM + D), BF16),
        in_specs=[hbm] * 14,
        out_specs=hbm,
        scratch_shapes=[
            pltpu.VMEM((3 * H + 2 * NSP, DM // 2, E), U32),
            pltpu.VMEM((H * E, DM), BF16) if True else pltpu.VMEM((DM // LANES, H * E // 2, LANES), U32),
            pltpu.VMEM((NSLOT, 3, DCH * (H // 2), E), U32),
            pltpu.VMEM((S, DM), BF16),
            pltpu.VMEM((S, DM), BF16),
            pltpu.VMEM((M + SEG, DM), F32),
            pltpu.VMEM((M + SEG, DM), F32),
            pltpu.VMEM((S, D), BF16),
            pltpu.VMEM((S, D), BF16),
            pltpu.VMEM((S, D), BF16),
            pltpu.VMEM((D, S), BF16),
            pltpu.VMEM((8 + CPS * CHUNK, LANES), F32),
            pltpu.VMEM((2, 2 * CHUNK, LANES), F32),
            pltpu.VMEM((2, NCH, 2 * CHUNK, LANES), F32),
            pltpu.VMEM((2, NCH, 2 * CHUNK, LANES), F32),
            pltpu.VMEM((3, NCH, 2 * CHUNK, LANES), F32),
            pltpu.VMEM((M, DM), BF16), pltpu.VMEM((KS, D), BF16), pltpu.VMEM((NCT, LANES), BF16),
            pltpu.VMEM((2 * CHUNK, CHUNK), BF16), pltpu.VMEM((CHUNK, 2 * CHUNK), BF16), dma((5,)),
            pltpu.VMEM((NCT, LANES), F32),
            dma((NSLOT, 3)), dma((NCT,)), dma((NCT + 2,)), dma((NCT + 2,)), dma((NCT + 2, 3)), dma, dma,
        ],
        compiler_params=pltpu.CompilerParams(vmem_limit_bytes=124 * 1024 * 1024,
                                             disable_bounds_checks='bc' not in DBG),
    )(
        A_mem0.reshape(M, DM), B_shift_k.T, B_ssm_D.reshape(NCT, LANES),
        jnp.asarray(_FWD, BF16), jnp.asarray(_INV, BF16),
        A_x.reshape(S, DM),
        A_Wq.reshape(DM * H, E), A_Wk.reshape(DM * H, E), A_Wv.reshape(DM * H, E),
        A_Wo.reshape(H * E, DM),
        B_q.reshape(S, D), B_k.reshape(S, D), B_v.reshape(S, D), B_ssm_k,
    )
    return out.reshape(B, S, DM + D)
```

```python
import functools

import jax
import jax.numpy as jnp
import numpy as np
import jax.experimental.pallas as pl
import jax.experimental.pallas.tpu as pltpu

BF16 = jnp.bfloat16
F32 = jnp.float32
U32 = jnp.uint32

LANES = 128
LOG2E = 1.4426950408889634
CHUNK = 128
NSLOT = 3
EARLY = 2
WO_DEPTH = 3

HEAD_ORDER = (("K", 0), ("P", 3), ("Q", 0), ("S", 1), ("V", 1), ("O", 4))
T_SPECTRA, D_SPECTRA = 13, 6
T_INVERSE = (32, 34)
T_PROD_PINNED = (2, 8)
T_PROD_FREE = (28, 29)
GRP = 2
N_PINNED = 10
KVP = 4


def _dft_tables():
    n = np.arange(CHUNK, dtype=np.float64)
    f = np.concatenate([np.arange(0, CHUNK, 2), np.arange(1, CHUNK, 2)]).astype(np.float64)
    theta = 2.0 * np.pi * (f[:, None] + 0.5) * n[None, :] / (2 * CHUNK)
    fwd = np.concatenate([np.cos(theta), -np.sin(theta)], axis=0)
    inv = np.concatenate([np.cos(theta).T, -np.sin(theta).T], axis=1) / CHUNK
    return fwd.astype(np.float32), inv.astype(np.float32)


_FWD, _INV = _dft_tables()


def _mult(x, n):
    return x if isinstance(x, int) else pl.multiple_of(x, n)


def _rem(x, n):
    return x % n if isinstance(x, int) else jax.lax.rem(x, n)


def _kernel(
    mem_hbm, shift_hbm, dvec_hbm, fwd_hbm, inv_hbm,
    x_hbm, wq_hbm, wk_hbm, wv_hbm, wo_hbm, bq_hbm, bk_hbm, bv_hbm, ssm_hbm,
    out_hbm,
    arena, wo, stage, xbuf, abuf, hbuf, accb,
    qb, kb, vb, sb, kf, xraw, xs, ks, ysf,
    mem_ref, shift_ref, dvec_ref, fwd_ref, inv_ref, sem_s, dvf,
    sem_w, sem_wo, sem_x, sem_q, sem_in, sem_ob, sem_a,
    *, S, DM, H, E, M, SEG, D, KS,
):
    L = M + SEG
    NSEG = S // SEG
    NCT = D // LANES
    NCH = S // CHUNK
    DCH = DM // NCT
    HP = H // 2
    NT = DM // LANES
    SPT = NSEG // NCT
    FPS = (CHUNK // 8) // SPT
    CPS = NCH // SPT
    XR = S // NCT
    HPP = H // NCT
    TR = DM // 2
    SPEC = 2 * CHUNK
    YPT = TR // SPEC
    NG = NCH // GRP

    wq32 = wq_hbm.bitcast(U32)
    wk32 = wk_hbm.bitcast(U32)
    wv32 = wv_hbm.bitcast(U32)

    def lanes_of(c):
        return pl.ds(_mult(c * LANES, LANES), LANES)

    def early_rows(part, per_step, total):
        return slice(0, EARLY * per_step) if part == 0 else slice(EARLY * per_step, total)

    def b_in_copies(c, part=None):
        col = lanes_of(c)
        if part is None:
            t, sem = slice(None), sem_in.at[c]
        else:
            t, sem = early_rows(part, CPS * CHUNK, S), sem_in.at[NCT + part]
        return (
            pltpu.make_async_copy(bk_hbm.at[t, col], kb.at[t, col], sem.at[0]),
            pltpu.make_async_copy(bv_hbm.at[t, col], vb.at[t, col], sem.at[1]),
            pltpu.make_async_copy(ssm_hbm.at[col, t], sb.at[col, t], sem.at[2]),
        )

    def xq_copies(c, part=None):
        if part is None:
            rows, t, sc = pl.ds(_mult(c * XR, XR), XR), slice(None), c
        else:
            rows, t, sc = early_rows(part, SEG, XR), early_rows(part, CPS * CHUNK, S), NCT + part
        return (
            pltpu.make_async_copy(x_hbm.at[rows, :], xbuf.at[rows, :], sem_x.at[sc]),
            pltpu.make_async_copy(bq_hbm.at[t, lanes_of(c)], qb.at[t, lanes_of(c)], sem_q.at[sc]),
        )

    def first_block_copies(part):
        return xq_copies(0, part) + b_in_copies(2, part)

    def w_copies(c, slot):
        rows = pl.ds(_mult(c * DCH * HP, DCH * HP), DCH * HP)
        return tuple(
            pltpu.make_async_copy(w.at[rows, :], stage.at[slot, i], sem_w.at[slot, i])
            for i, w in enumerate((wq32, wk32, wv32))
        )

    def wo_copy(p):
        rows = pl.ds(_mult(p * HPP * E, HPP * E), HPP * E)
        return pltpu.make_async_copy(wo_hbm.at[rows, :], wo.at[rows, :], sem_wo.at[p])

    def send_outputs(s, c, part):
        rows = pl.ds(_mult(s * SEG, SEG), SEG)
        pltpu.make_async_copy(abuf.at[rows, :], out_hbm.at[rows, pl.ds(0, DM)], sem_a).start()
        rows = pl.ds(_mult(part * CPS * CHUNK, CPS * CHUNK), CPS * CHUNK)
        pltpu.make_async_copy(
            qb.at[rows, lanes_of(c)], out_hbm.at[rows, lanes_of(NT + c)], sem_ob).start()

    def wait_block_inputs(c):
        for cp in xq_copies(c):
            cp.wait()

        @pl.when(c + 2 < NCT)
        def _():
            for cp in b_in_copies(c + 2):
                cp.wait()

    def relayout(c, slot, i):
        r0 = _mult(c * (DCH // 2), DCH // 2)

        def repack(words):
            return pltpu.bitcast(pltpu.bitcast(words, F32).astype(BF16), U32)

        for j in range(HP):
            for dd in range(DCH // 16):
                a = stage[slot, i, pl.ds(dd * 16 * HP + j, 8, stride=HP), :]
                b = stage[slot, i, pl.ds((dd * 16 + 8) * HP + j, 8, stride=HP), :]
                ab = jnp.concatenate([a, b], axis=0)
                dst = pl.ds(r0 + dd * 8, 8)
                arena[3 * (2 * j) + i, dst, :] = repack(ab << 16)
                arena[3 * (2 * j + 1) + i, dst, :] = repack(ab & jnp.uint32(0xFFFF0000))

    def weight(head, i):
        return pltpu.bitcast(arena[3 * head + i], BF16)

    def y_rows(slot, j, r, n):
        tile = 3 * H + slot * (NCH // YPT) + j // YPT
        return tile, pl.ds(_mult((j % YPT) * SPEC + r, 8), n)

    def conv_taps(c):
        return shift_ref[:, lanes_of(c)].astype(F32)

    def stage_k(c, part):
        n = CPS * CHUNK
        kf[0:8, :] = jnp.where(part == 0, 0.0, kf[n:n + 8, :])
        kf[8:n + 8, :] = kb[pl.ds(_mult(part * n, n), n), lanes_of(c)].astype(F32)

    def kv_piece(c, part, u, taps, piece):
        n = CHUNK // KVP
        j = part * CPS + u
        rows = pl.ds(_mult(j * CHUNK + piece * n, n), n)
        k0 = u * CHUNK + piece * n + 8
        acc = kf[k0:k0 + n, :] * taps[0:1, :]
        for t in range(1, KS):
            acc = acc + kf[k0 - t:k0 - t + n, :] * taps[t:t + 1, :]
        kv = (acc * vb[rows, lanes_of(c)].astype(F32)).astype(BF16)
        vb[rows, lanes_of(c)] = kv
        return kv

    def x_spectrum(slot, part, u, kv):
        j = part * CPS + u
        half = CHUNK // 2
        xj = jnp.dot(fwd_ref[...], kv, preferred_element_type=F32)
        prev = xraw[u % 2]
        if u == 0:
            prev = jnp.where(part == 0, 0.0, prev)
        xraw[1 - u % 2] = xj
        xs[slot, j, 0:half, :] = xj[0:half] - prev[CHUNK:CHUNK + half]
        xs[slot, j, half:CHUNK, :] = xj[half:CHUNK] + prev[CHUNK + half:]
        xs[slot, j, CHUNK:CHUNK + half, :] = xj[CHUNK:CHUNK + half] + prev[0:half]
        xs[slot, j, CHUNK + half:, :] = xj[CHUNK + half:] - prev[half:CHUNK]

    def k_spectrum(c, slot, part, u):
        j = part * CPS + u
        blk = sb[lanes_of(c), pl.ds(_mult(j * CHUNK, CHUNK), CHUNK)]
        ks[slot, j] = jax.lax.dot_general(
            fwd_ref[...], blk, (((1,), (1,)), ((), ())), preferred_element_type=F32)

    def is_free(f, ig):
        return f * NG + ig >= N_PINNED

    def products(slot, fb, ig, free):
        r = _mult(fb * 8, 8)
        re, im = pl.ds(r, 8), pl.ds(r + CHUNK, 8)
        accs = [None] * GRP
        xv = {}
        for m in range(GRP * ig + GRP):
            kr = ks[slot, m, re, :]
            ki = ks[slot, m, im, :]
            for u in range(GRP):
                j = GRP * ig + u - m
                if j < 0:
                    continue
                if j not in xv:
                    xv[j] = (xs[slot, j, re, :], xs[slot, j, im, :])
                xr, xi = xv[j]
                if accs[u] is None:
                    accs[u] = (kr * xr - ki * xi, kr * xi + ki * xr)
                else:
                    ar, ai = accs[u]
                    accs[u] = (ar + kr * xr - ki * xi, ai + kr * xi + ki * xr)
            yield
        for u in range(GRP):
            i = GRP * ig + u
            if free:
                ysf[slot, i, re, :] = accs[u][0]
                ysf[slot, i, im, :] = accs[u][1]
            else:
                tile, rows = y_rows(slot, i, r, 8)
                arena[tile, rows, :] = pltpu.bitcast(accs[u][0], U32)
                tile, rows = y_rows(slot, i, r + CHUNK, 8)
                arena[tile, rows, :] = pltpu.bitcast(accs[u][1], U32)

    def inverse(c, slot, i):
        cols = lanes_of(c)
        rows = pl.ds(_mult(i * CHUNK, CHUNK), CHUNK)
        dvec = dvf[pl.ds(c, 1), :]
        tile, yrows = y_rows(slot, i, 0, SPEC)
        ya = pltpu.bitcast(arena[tile, yrows, :], F32)
        yb = ysf[slot, i]
        pieces = []
        for blk in range(SPEC // 8):
            f = (blk % (CHUNK // 8)) % FPS
            rows8 = slice(blk * 8, blk * 8 + 8)
            pinned = sum(not is_free(f, ig) for ig in range(NG))
            if pinned == 0:
                pieces.append(yb[rows8])
            elif pinned == NG:
                pieces.append(ya[rows8])
            else:
                pieces.append(jnp.where(i < pinned * GRP, ya[rows8], yb[rows8]))
        yy = jnp.concatenate(pieces, axis=0)
        y = jnp.dot(inv_ref[...], yy.astype(BF16), preferred_element_type=F32)
        kv = vb[rows, cols].astype(F32)
        qv = qb[rows, cols].astype(F32)
        qb[rows, cols] = (qv * (y + kv * dvec)).astype(BF16)

    small = [pltpu.make_async_copy(a, b, sem_s.at[i]) for i, (a, b) in enumerate(
        ((mem_hbm, mem_ref), (shift_hbm, shift_ref), (dvec_hbm, dvec_ref),
         (fwd_hbm, fwd_ref), (inv_hbm, inv_ref)))]
    for c0 in range(NSLOT - 1):
        for cp in w_copies(c0, c0):
            cp.start()
    for cp in small:
        cp.start()
    for c0 in range(2):
        for cp in b_in_copies(c0):
            cp.start()
    for cp in first_block_copies(0):
        cp.start()
    for cp in small:
        cp.wait()
    dvf[...] = dvec_ref[...].astype(F32)

    def pro_iter(c, carry):
        slot = jax.lax.rem(c, NSLOT)
        ahead = c + NSLOT - 1

        @pl.when(ahead < NCT)
        def _():
            for cp in w_copies(ahead, jax.lax.rem(ahead, NSLOT)):
                cp.start()

        for cc, lo, hi in ((NCT - NSLOT, 0, 1), (NCT - NSLOT + 1, 1, WO_DEPTH)):
            @pl.when(c == cc)
            def _(lo=lo, hi=hi):
                for p in range(lo, hi):
                    wo_copy(p).start()

        for i, cp in enumerate(w_copies(c, slot)):
            cp.wait()
            relayout(c, slot, i)

        @pl.when((c == 2) | (c == 3))
        def _():
            for cp in b_in_copies(c - 2):
                cp.wait()
            taps = conv_taps(c - 2)

            def spectra_part(part, z):
                stage_k(c - 2, part)
                for u in range(CPS):
                    kv = jnp.concatenate(
                        [kv_piece(c - 2, part, u, taps, q) for q in range(KVP)], axis=0)
                    x_spectrum(c - 2, part, u, kv)
                    k_spectrum(c - 2, c - 2, part, u)
                return z

            jax.lax.fori_loop(0, SPT, spectra_part, 0)

        @pl.when(c == 4)
        def _():
            def body(fb, z):
                for f in range(FPS):
                    for ig in range(NG):
                        for _ in products(0, fb * FPS + f, ig, is_free(f, ig)):
                            pass
                return z

            jax.lax.fori_loop(0, SPT, body, 0)

        return carry

    jax.lax.fori_loop(0, NCT, pro_iter, 0)

    row = jax.lax.broadcasted_iota(jnp.int32, (L, L), 0)
    col = jax.lax.broadcasted_iota(jnp.int32, (L, L), 1)
    mask = (row < M) | (row >= col)
    scale = E ** -0.5
    hbuf[0:M, :] = mem_ref[...].astype(F32)

    maxlag = max(lag for _, lag in HEAD_ORDER)
    ops = [(op, t - lag, t) for t in range(H + maxlag + 1) for op, lag in HEAD_ORDER
           if 0 <= t - lag < H]

    def slot_of(t, op="O"):
        for n, (o, _, tt) in enumerate(ops):
            if tt > t or (tt == t and o == op):
                return n
        return len(ops)

    def segment(s, first=False):
        c = s // SPT
        part = s % SPT
        c2 = _rem(c + 2, NCT)
        par = _rem(c, 2)

        side = {}
        st = {}

        def at(n, fn):
            side.setdefault(min(n, len(ops)), []).append(fn)

        at(slot_of(T_SPECTRA), lambda: (stage_k(c2, part), st.update(taps=conv_taps(c2))))
        for u in range(CPS):
            nu = slot_of(T_SPECTRA + 1 + u * D_SPECTRA)
            for q in range(KVP):
                at(nu + q, lambda u=u, q=q: st.update(
                    {(u, q): kv_piece(c2, part, u, st["taps"], q)}))
            nx = max(slot_of(T_SPECTRA + 2 + u * D_SPECTRA, "K"), nu + KVP - 1)
            at(nx, lambda u=u: x_spectrum(par, part, u, jnp.concatenate(
                [st.pop((u, q)) for q in range(KVP)], axis=0)))
            at(nx + 1, lambda u=u: k_spectrum(c2, par, part, u))
        for u in range(CPS):
            at(slot_of(T_INVERSE[u], "Q"), functools.partial(inverse, c, par, part * CPS + u))

        def prod_stream(free):
            for n in range(FPS * NG):
                f, ig = n // NG, n % NG
                if is_free(f, ig) == free:
                    yield from products(1 - par, part * FPS + f, ig, free)
                    yield

        for free, (t0, t1) in ((False, T_PROD_PINNED), (True, T_PROD_FREE)):
            gen = prod_stream(free)
            nmicro = sum(GRP * ig + GRP + 1 for f in range(FPS) for ig in range(NG)
                         if is_free(f, ig) == free)
            p0, p1 = slot_of(t0), slot_of(t1)
            for n in range(nmicro):
                at(p0 + n * (p1 - p0) // nmicro, lambda gen=gen: next(gen, None))

        r0 = _mult(s * SEG, SEG)
        hbuf[M:L, :] = xbuf[pl.ds(r0, SEG), :].astype(F32)
        h = hbuf[...]
        Q, K, V, P, O, Z = {}, {}, {}, {}, {}, {}
        acc = [None] * NT

        for n, (op, hd, _) in enumerate(ops):
            for fn in side.pop(n, []):
                fn()
            if op == "Q":
                Q[hd] = jnp.dot(h, weight(hd, 0), preferred_element_type=F32)
            elif op == "K":
                K[hd] = jnp.dot(h, weight(hd, 1), preferred_element_type=F32).astype(BF16)
            elif op == "V":
                V[hd] = jnp.dot(h, weight(hd, 2), preferred_element_type=F32).astype(BF16)
            elif op == "S":
                sc = jax.lax.dot_general(Q.pop(hd), K.pop(hd), (((1,), (1,)), ((), ())),
                                         preferred_element_type=F32)
                sc = jnp.where(mask, sc, -1e9 / scale)
                p = jnp.exp2((sc - jnp.max(sc, axis=-1, keepdims=True)) * (scale * LOG2E))
                P[hd] = p
                Z[hd] = jnp.sum(p, axis=-1, keepdims=True)
            elif op == "P":
                z = Z.pop(hd)
                r = pltpu.reciprocal(z, approx=True)
                r = r * (2.0 - z * r)
                O[hd] = jnp.dot(P.pop(hd), V.pop(hd), preferred_element_type=F32) * r
            else:
                if first and hd % HPP == 0:
                    wo_copy(hd // HPP).wait()
                    if hd // HPP + WO_DEPTH < NCT:
                        wo_copy(hd // HPP + WO_DEPTH).start()
                    if hd == H - HPP:
                        for cp in first_block_copies(1):
                            cp.start()
                o = O.pop(hd)
                for nn in range(NT):
                    cols = slice(nn * LANES, (nn + 1) * LANES)
                    y = jnp.dot(o, wo[hd * E:(hd + 1) * E, cols], preferred_element_type=F32)
                    if hd == 0:
                        accb[:, cols] = y
                    elif hd < H - 1:
                        accb[:, cols] += y
                    else:
                        acc[nn] = accb[:, cols] + y
        for fn in side.pop(len(ops), []):
            fn()
        out = jnp.concatenate(acc, axis=1).astype(BF16)
        hbuf[0:M, :] = out[0:M].astype(F32)
        abuf[pl.ds(r0, SEG), :] = out[M:L]
        send_outputs(s, c, part)
        nxt = s + 1

        @pl.when((nxt % SPT == 0) & (nxt < NSEG))
        def _():
            wait_block_inputs(nxt // SPT)

    for cp in first_block_copies(0):
        cp.wait()
    for s0 in range(EARLY):
        segment(s0, first=(s0 == 0))
    for cp in first_block_copies(1):
        cp.wait()
    for c0 in range(1, NCT):
        for cp in xq_copies(c0):
            cp.start()
        if c0 >= 3:
            for cp in b_in_copies(c0):
                cp.start()

    def steps(i, carry):
        segment(EARLY + i)
        return carry

    jax.lax.fori_loop(0, NSEG - EARLY, steps, 0)

    pltpu.make_async_copy(qb, qb, sem_ob).wait()
    pltpu.make_async_copy(abuf, out_hbm.at[:, pl.ds(0, DM)], sem_a).wait()


@functools.partial(jax.jit, static_argnames=("A_seg_len",))
def pallas_concat_heads__memory_aug_recurrent_mem_tr__ssm_conv_h3__prompt_kernel(
    A_x: jax.Array,
    A_mem0: jax.Array,
    A_Wq: jax.Array,
    A_Wk: jax.Array,
    A_Wv: jax.Array,
    A_Wo: jax.Array,
    A_seg_len: int,
    B_q: jax.Array,
    B_k: jax.Array,
    B_v: jax.Array,
    B_shift_k: jax.Array,
    B_ssm_k: jax.Array,
    B_ssm_D: jax.Array,
):
    B, S, DM = A_x.shape
    H, E = A_Wq.shape[1], A_Wq.shape[2]
    M = A_mem0.shape[1]
    SEG = int(A_seg_len)
    D = B_q.shape[2]
    KS = B_shift_k.shape[1]
    NCT = D // LANES
    NCH = S // CHUNK
    DCH = DM // NCT
    NSEG = S // SEG
    assert B == 1 and E == LANES and M == 8 and KS <= 8
    assert S % CHUNK == 0 and S % SEG == 0 and NSEG % NCT == 0 and NCH % (NSEG // NCT) == 0
    assert H % NCT == 0 and DCH % 16 == 0 and (CHUNK // 8) % (NSEG // NCT) == 0
    CPS = NCH // (NSEG // NCT)
    NSP = NCH * 2 * CHUNK // (DM // 2)

    kernel = functools.partial(_kernel, S=S, DM=DM, H=H, E=E, M=M, SEG=SEG, D=D, KS=KS)
    hbm = pl.BlockSpec(memory_space=pl.ANY)
    dma = pltpu.SemaphoreType.DMA

    out = pl.pallas_call(
        kernel,
        out_shape=jax.ShapeDtypeStruct((S, DM + D), BF16),
        in_specs=[hbm] * 14,
        out_specs=hbm,
        scratch_shapes=[
            pltpu.VMEM((3 * H + 2 * NSP, DM // 2, E), U32),
            pltpu.VMEM((H * E, DM), BF16),
            pltpu.VMEM((NSLOT, 3, DCH * (H // 2), E), U32),
            pltpu.VMEM((S, DM), BF16),
            pltpu.VMEM((S, DM), BF16),
            pltpu.VMEM((M + SEG, DM), F32),
            pltpu.VMEM((M + SEG, DM), F32),
            pltpu.VMEM((S, D), BF16),
            pltpu.VMEM((S, D), BF16),
            pltpu.VMEM((S, D), BF16),
            pltpu.VMEM((D, S), BF16),
            pltpu.VMEM((8 + CPS * CHUNK, LANES), F32),
            pltpu.VMEM((2, 2 * CHUNK, LANES), F32),
            pltpu.VMEM((2, NCH, 2 * CHUNK, LANES), F32),
            pltpu.VMEM((2, NCH, 2 * CHUNK, LANES), F32),
            pltpu.VMEM((2, NCH, 2 * CHUNK, LANES), F32),
            pltpu.VMEM((M, DM), BF16),
            pltpu.VMEM((KS, D), BF16),
            pltpu.VMEM((NCT, LANES), BF16),
            pltpu.VMEM((2 * CHUNK, CHUNK), BF16),
            pltpu.VMEM((CHUNK, 2 * CHUNK), BF16),
            dma((5,)),
            pltpu.VMEM((NCT, LANES), F32),
            dma((NSLOT, 3)), dma((NCT,)), dma((NCT + 2,)), dma((NCT + 2,)), dma((NCT + 2, 3)),
            dma, dma,
        ],
        compiler_params=pltpu.CompilerParams(
            vmem_limit_bytes=124 * 1024 * 1024, disable_bounds_checks=True),
    )(
        A_mem0.reshape(M, DM), B_shift_k.T, B_ssm_D.reshape(NCT, LANES),
        jnp.asarray(_FWD, BF16), jnp.asarray(_INV, BF16),
        A_x.reshape(S, DM),
        A_Wq.reshape(DM * H, E), A_Wk.reshape(DM * H, E), A_Wv.reshape(DM * H, E),
        A_Wo.reshape(H * E, DM),
        B_q.reshape(S, D), B_k.reshape(S, D), B_v.reshape(S, D), B_ssm_k,
    )
    return out.reshape(B, S, DM + D)
```

```python
import functools

import jax
import jax.numpy as jnp
import numpy as np
import jax.experimental.pallas as pl
import jax.experimental.pallas.tpu as pltpu

BF16 = jnp.bfloat16
F32 = jnp.float32
U32 = jnp.uint32

LANES = 128
LOG2E = 1.4426950408889634
CHUNK = 128
NSLOT = 5
EARLY = 2
NPRE = 5
WO_DEPTH = 3

HEAD_ORDER = (("K", 0), ("P", 3), ("Q", 0), ("S", 1), ("V", 1), ("O", 4))
HEAD_ORDER_PRE = (("K", 0), ("P", 3), ("V", 1), ("Q", 0), ("S", 1), ("O", 4))
T_SPECTRA, D_SPECTRA = 15, 6
T_INVERSE = (32, 33)
T_PROD_PINNED = (2, 8)
T_PROD_FREE = (28, 29)
GRP = 2
N_PINNED = 10
KVP = 4


def _dft_tables():
    n = np.arange(CHUNK, dtype=np.float64)
    f = np.concatenate([np.arange(0, CHUNK, 2), np.arange(1, CHUNK, 2)]).astype(np.float64)
    theta = 2.0 * np.pi * (f[:, None] + 0.5) * n[None, :] / (2 * CHUNK)
    fwd = np.concatenate([np.cos(theta), -np.sin(theta)], axis=0)
    inv = np.concatenate([np.cos(theta).T, -np.sin(theta).T], axis=1) / CHUNK
    return fwd.astype(np.float32), inv.astype(np.float32)


_FWD, _INV = _dft_tables()


def _mult(x, n):
    return x if isinstance(x, int) else pl.multiple_of(x, n)


def _rem(x, n):
    return x % n if isinstance(x, int) else jax.lax.rem(x, n)


def _kernel(
    mem_hbm, shift_hbm, dvec_hbm, fwd_hbm, inv_hbm,
    x_hbm, wq_hbm, wk_hbm, wv_hbm, wo_hbm, bq_hbm, bk_hbm, bv_hbm, ssm_hbm,
    out_hbm,
    arena, wo, stage, xbuf, abuf, hbuf, accb, pre,
    qb, kb, vb, sb, kf, xraw, xs, ks, ysf,
    mem_ref, shift_ref, dvec_ref, fwd_ref, inv_ref, sem_s, dvf,
    sem_w, sem_wo, sem_x, sem_q, sem_in, sem_ob, sem_a,
    *, S, DM, H, E, M, SEG, D, KS,
):
    L = M + SEG
    NSEG = S // SEG
    NCT = D // LANES
    NCH = S // CHUNK
    DCH = DM // NCT
    HP = H // 2
    NT = DM // LANES
    SPT = NSEG // NCT
    FPS = (CHUNK // 8) // SPT
    CPS = NCH // SPT
    XR = S // NCT
    HPP = H // NCT
    TR = DM // 2
    SPEC = 2 * CHUNK
    YPT = TR // SPEC
    NG = NCH // GRP

    wq32 = wq_hbm.bitcast(U32)
    wk32 = wk_hbm.bitcast(U32)
    wv32 = wv_hbm.bitcast(U32)

    def lanes_of(c):
        return pl.ds(_mult(c * LANES, LANES), LANES)

    def early_rows(part, per_step, total):
        return slice(0, EARLY * per_step) if part == 0 else slice(EARLY * per_step, total)

    def b_in_copies(c, part=None):
        col = lanes_of(c)
        if part is None:
            t, sem = slice(None), sem_in.at[c]
        else:
            t, sem = early_rows(part, CPS * CHUNK, S), sem_in.at[NCT + part]
        return (
            pltpu.make_async_copy(bk_hbm.at[t, col], kb.at[t, col], sem.at[0]),
            pltpu.make_async_copy(bv_hbm.at[t, col], vb.at[t, col], sem.at[1]),
            pltpu.make_async_copy(ssm_hbm.at[col, t], sb.at[col, t], sem.at[2]),
        )

    def x_copy(c):
        rows = pl.ds(_mult(c * XR, XR), XR)
        return pltpu.make_async_copy(x_hbm.at[rows, :], xbuf.at[rows, :], sem_x.at[c])

    def q_copy(c, part=None):
        t, sc = (slice(None), c) if part is None else (early_rows(part, CPS * CHUNK, S), NCT + part)
        return pltpu.make_async_copy(bq_hbm.at[t, lanes_of(c)], qb.at[t, lanes_of(c)], sem_q.at[sc])

    def xq_copies(c):
        return (x_copy(c), q_copy(c))

    def first_block_copies(part):
        return (q_copy(0, part),) + b_in_copies(2, part)

    def w_copy(g, slot):
        i, c = g
        rows = pl.ds(_mult(c * DCH * HP, DCH * HP), DCH * HP)
        return pltpu.make_async_copy((wq32, wk32, wv32)[i].at[rows, :], stage.at[slot], sem_w.at[slot])

    def wo_copy(p):
        rows = pl.ds(_mult(p * HPP * E, HPP * E), HPP * E)
        return pltpu.make_async_copy(wo_hbm.at[rows, :], wo.at[rows, :], sem_wo.at[p])

    def send_outputs(s, c, part):
        rows = pl.ds(_mult(s * SEG, SEG), SEG)
        pltpu.make_async_copy(abuf.at[rows, :], out_hbm.at[rows, pl.ds(0, DM)], sem_a).start()
        rows = pl.ds(_mult(part * CPS * CHUNK, CPS * CHUNK), CPS * CHUNK)
        pltpu.make_async_copy(
            qb.at[rows, lanes_of(c)], out_hbm.at[rows, lanes_of(NT + c)], sem_ob).start()

    def wait_block_inputs(c):
        for cp in xq_copies(c):
            cp.wait()

        @pl.when(c + 2 < NCT)
        def _():
            for cp in b_in_copies(c + 2):
                cp.wait()

    def relayout(c, slot, i, j0, j1):
        r0 = _mult(c * (DCH // 2), DCH // 2)

        def repack(words):
            return pltpu.bitcast(pltpu.bitcast(words, F32).astype(BF16), U32)

        for j in range(j0, j1):
            for dd in range(DCH // 16):
                a = stage[slot, pl.ds(dd * 16 * HP + j, 8, stride=HP), :]
                b = stage[slot, pl.ds((dd * 16 + 8) * HP + j, 8, stride=HP), :]
                ab = jnp.concatenate([a, b], axis=0)
                dst = pl.ds(r0 + dd * 8, 8)
                arena[3 * (2 * j) + i, dst, :] = repack(ab << 16)
                arena[3 * (2 * j + 1) + i, dst, :] = repack(ab & jnp.uint32(0xFFFF0000))

    def weight(head, i):
        return pltpu.bitcast(arena[3 * head + i], BF16)

    def y_rows(slot, j, r, n):
        tile = 3 * H + slot * (NCH // YPT) + j // YPT
        return tile, pl.ds(_mult((j % YPT) * SPEC + r, 8), n)

    def conv_taps(c):
        return shift_ref[:, lanes_of(c)].astype(F32)

    def stage_k(c, part, b=0):
        n = CPS * CHUNK
        kf[b, 0:8, :] = jnp.where(part == 0, 0.0, kf[b, n:n + 8, :])
        kf[b, 8:n + 8, :] = kb[pl.ds(_mult(part * n, n), n), lanes_of(c)].astype(F32)

    def kv_piece(c, part, u, taps, piece, b=0):
        n = CHUNK // KVP
        j = part * CPS + u
        rows = pl.ds(_mult(j * CHUNK + piece * n, n), n)
        k0 = u * CHUNK + piece * n + 8
        acc = kf[b, k0:k0 + n, :] * taps[0:1, :]
        for t in range(1, KS):
            acc = acc + kf[b, k0 - t:k0 - t + n, :] * taps[t:t + 1, :]
        kv = (acc * vb[rows, lanes_of(c)].astype(F32)).astype(BF16)
        vb[rows, lanes_of(c)] = kv
        return kv

    def x_spectrum(slot, part, u, kv, b=0):
        j = part * CPS + u
        half = CHUNK // 2
        xj = jnp.dot(fwd_ref[...], kv, preferred_element_type=F32)
        prev = xraw[2 * b + u % 2]
        if u == 0:
            prev = jnp.where(part == 0, 0.0, prev)
        xraw[2 * b + 1 - u % 2] = xj
        xs[slot, j, 0:half, :] = xj[0:half] - prev[CHUNK:CHUNK + half]
        xs[slot, j, half:CHUNK, :] = xj[half:CHUNK] + prev[CHUNK + half:]
        xs[slot, j, CHUNK:CHUNK + half, :] = xj[CHUNK:CHUNK + half] + prev[0:half]
        xs[slot, j, CHUNK + half:, :] = xj[CHUNK + half:] - prev[half:CHUNK]

    def k_spectrum(c, slot, part, u):
        j = part * CPS + u
        blk = sb[lanes_of(c), pl.ds(_mult(j * CHUNK, CHUNK), CHUNK)]
        ks[slot, j] = jax.lax.dot_general(
            fwd_ref[...], blk, (((1,), (1,)), ((), ())), preferred_element_type=F32)

    def is_free(f, ig):
        return f * NG + ig >= N_PINNED

    def products(slot, fb, ig, free):
        r = _mult(fb * 8, 8)
        re, im = pl.ds(r, 8), pl.ds(r + CHUNK, 8)
        accs = [None] * GRP
        xv = {}
        for m in range(GRP * ig + GRP):
            kr = ks[slot, m, re, :]
            ki = ks[slot, m, im, :]
            for u in range(GRP):
                j = GRP * ig + u - m
                if j < 0:
                    continue
                if j not in xv:
                    xv[j] = (xs[slot, j, re, :], xs[slot, j, im, :])
                xr, xi = xv[j]
                if accs[u] is None:
                    accs[u] = (kr * xr - ki * xi, kr * xi + ki * xr)
                else:
                    ar, ai = accs[u]
                    accs[u] = (ar + kr * xr - ki * xi, ai + kr * xi + ki * xr)
            yield
        for u in range(GRP):
            i = GRP * ig + u
            if free:
                ysf[slot, i, re, :] = accs[u][0]
                ysf[slot, i, im, :] = accs[u][1]
            else:
                tile, rows = y_rows(slot, i, r, 8)
                arena[tile, rows, :] = pltpu.bitcast(accs[u][0], U32)
                tile, rows = y_rows(slot, i, r + CHUNK, 8)
                arena[tile, rows, :] = pltpu.bitcast(accs[u][1], U32)

    def inverse(c, slot, i):
        cols = lanes_of(c)
        rows = pl.ds(_mult(i * CHUNK, CHUNK), CHUNK)
        dvec = dvf[pl.ds(c, 1), :]
        tile, yrows = y_rows(slot, i, 0, SPEC)
        ya = pltpu.bitcast(arena[tile, yrows, :], F32)
        yb = ysf[slot, i]
        pieces = []
        for blk in range(SPEC // 8):
            f = (blk % (CHUNK // 8)) % FPS
            rows8 = slice(blk * 8, blk * 8 + 8)
            pinned = sum(not is_free(f, ig) for ig in range(NG))
            if pinned == 0:
                pieces.append(yb[rows8])
            elif pinned == NG:
                pieces.append(ya[rows8])
            else:
                pieces.append(jnp.where(i < pinned * GRP, ya[rows8], yb[rows8]))
        yy = jnp.concatenate(pieces, axis=0)
        y = jnp.dot(inv_ref[...], yy.astype(BF16), preferred_element_type=F32)
        kv = vb[rows, cols].astype(F32)
        qv = qb[rows, cols].astype(F32)
        qb[rows, cols] = (qv * (y + kv * dvec)).astype(BF16)

    small = [pltpu.make_async_copy(a, b, sem_s.at[i]) for i, (a, b) in enumerate(
        ((mem_hbm, mem_ref), (shift_hbm, shift_ref), (dvec_hbm, dvec_ref),
         (fwd_hbm, fwd_ref), (inv_hbm, inv_ref)))]
    for cp in small:
        cp.start()
    for cp in b_in_copies(0):
        cp.start()
    for cp in small:
        cp.wait()
    for cp in b_in_copies(0):
        cp.wait()
    for cp in b_in_copies(1):
        cp.start()
    for g in range(NSLOT - 1):
        w_copy((g // NCT, g % NCT), g).start()
    x_copy(0).start()
    for cp in first_block_copies(0):
        cp.start()
    dvf[...] = dvec_ref[...].astype(F32)

    def precompute(i, hd0, nh):
        xs_ = xbuf[SEG:(NPRE + 1) * SEG, :]
        for hh in range(nh):
            hd = hd0 + hh
            pre[i, :, pl.ds(_mult(hd * E, E), E)] = jnp.dot(
                xs_, weight(hd, i), preferred_element_type=F32).astype(BF16)

    def lead_products(part, f, ig):
        for _ in products(0, part * FPS + f, ig, is_free(f, ig)):
            pass

    def weight_phase(i):
        def body(c, carry):
            g = i * NCT + c
            slot = jax.lax.rem(g, NSLOT)
            ahead = c + NSLOT - 1
            nslot = jax.lax.rem(g + NSLOT - 1, NSLOT)

            @pl.when(ahead < NCT)
            def _():
                w_copy((i, ahead), nslot).start()

            if i < 2:
                @pl.when(ahead >= NCT)
                def _():
                    w_copy((i + 1, ahead - NCT), nslot).start()
            else:
                for p in range(WO_DEPTH):
                    @pl.when(c == NCT - WO_DEPTH + p)
                    def _(p=p):
                        wo_copy(p).start()
            w_copy((i, c), slot).wait()
            jobs = [[] for _ in range(HPP)]
            if i == 0:
                st = {}
                for b in range(2):
                    for u in range(CPS):
                        jobs[0].append(functools.partial(k_spectrum, b, b, c, u))
                for b in range(2):
                    jobs[0].append(functools.partial(stage_k, b, c, b))
                for b in range(2):
                    for u in range(CPS):
                        jobs[min(2 * b + u, 1)].append(lambda b=b, u=u: st.update({(b, u): jnp.concatenate(
                            [kv_piece(b, c, u, conv_taps(b), q, b) for q in range(KVP)], axis=0)}))
                for b in range(2):
                    for u in range(CPS):
                        jobs[2].append(lambda b=b, u=u: x_spectrum(b, c, u, st.pop((b, u)), b))
            elif i == 1:
                for n in range(FPS * NG):
                    jobs[n * HPP // (FPS * NG)].append(
                        functools.partial(lead_products, c, n // NG, n % NG))
            for hh in range(HPP):
                for fn in jobs[hh]:
                    fn()
                if i >= 1:
                    precompute(i - 1, c * HPP + hh, 1)
                relayout(c, slot, i, hh * HP // HPP, (hh + 1) * HP // HPP)
            return carry

        jax.lax.fori_loop(0, NCT, body, 0)

    for i in range(3):
        if i == 0:
            for cp in b_in_copies(1):
                cp.wait()
        if i == 1:
            x_copy(0).wait()
        weight_phase(i)

    row = jax.lax.broadcasted_iota(jnp.int32, (L, L), 0)
    col = jax.lax.broadcasted_iota(jnp.int32, (L, L), 1)
    mask = (row < M) | (row >= col)
    scale = E ** -0.5
    hbuf[0:M, :] = mem_ref[...].astype(F32)

    def start_late():
        for c0 in range(1, NCT):
            for cp in xq_copies(c0):
                cp.start()
            if c0 >= 3:
                for cp in b_in_copies(c0):
                    cp.start()

    def segment(s, first=False, fast=False):
        order = HEAD_ORDER_PRE if fast else HEAD_ORDER
        maxlag = max(lag for _, lag in order)
        ops = [(op, t - lag, t) for t in range(H + maxlag + 1) for op, lag in order
               if 0 <= t - lag < H]

        def slot_of(t, op="O"):
            for n, (o, _, tt) in enumerate(ops):
                if tt > t or (tt == t and o == op):
                    return n
            return len(ops)

        c = s // SPT
        part = s % SPT
        c2 = _rem(c + 2, NCT)
        par = _rem(c, 2)

        side = {}
        st = {}

        def at(n, fn):
            side.setdefault(min(n, len(ops)), []).append(fn)

        at(slot_of(T_SPECTRA), lambda: (stage_k(c2, part), st.update(taps=conv_taps(c2))))
        for u in range(CPS):
            nu = slot_of(T_SPECTRA + 1 + u * D_SPECTRA)
            for q in range(KVP):
                at(nu + q, lambda u=u, q=q: st.update(
                    {(u, q): kv_piece(c2, part, u, st["taps"], q)}))
            nx = max(slot_of(T_SPECTRA + 2 + u * D_SPECTRA, "K"), nu + KVP - 1)
            at(nx, lambda u=u: x_spectrum(par, part, u, jnp.concatenate(
                [st.pop((u, q)) for q in range(KVP)], axis=0)))
            at(nx + 1, lambda u=u: k_spectrum(c2, par, part, u))
        for u in range(CPS):
            at(slot_of(T_INVERSE[u], "Q"), functools.partial(inverse, c, par, part * CPS + u))

        def prod_stream(free):
            for n in range(FPS * NG):
                f, ig = n // NG, n % NG
                if is_free(f, ig) == free:
                    yield from products(1 - par, part * FPS + f, ig, free)
                    yield

        for free, (t0, t1) in ((False, T_PROD_PINNED), (True, T_PROD_FREE)):
            gen = prod_stream(free)
            nmicro = sum(GRP * ig + GRP + 1 for f in range(FPS) for ig in range(NG)
                         if is_free(f, ig) == free)
            p0, p1 = slot_of(t0), slot_of(t1)
            for n in range(nmicro):
                at(p0 + n * (p1 - p0) // nmicro, lambda gen=gen: next(gen, None))

        r0 = _mult(s * SEG, SEG)
        hbuf[M:L, :] = xbuf[pl.ds(r0, SEG), :].astype(F32)
        h = hbuf[...]
        Q, K, V, P, O, Z = {}, {}, {}, {}, {}, {}
        acc = [None] * NT

        for n, (op, hd, _) in enumerate(ops):
            for fn in side.pop(n, []):
                fn()
            if op in "QK":
                i = "QK".index(op)
                if fast:
                    rows = pl.ds(_mult((s - 1) * SEG, SEG), SEG)
                    res = jnp.concatenate([
                        jnp.dot(hbuf[0:M, :], weight(hd, i), preferred_element_type=F32),
                        pre[i, rows, hd * E:(hd + 1) * E].astype(F32)], axis=0)
                else:
                    res = jnp.dot(h, weight(hd, i), preferred_element_type=F32)
                if op == "Q":
                    Q[hd] = res
                else:
                    K[hd] = res.astype(BF16)
            elif op == "V":
                V[hd] = jnp.dot(h, weight(hd, 2), preferred_element_type=F32).astype(BF16)
            elif op == "S":
                sc = jax.lax.dot_general(Q.pop(hd), K.pop(hd), (((1,), (1,)), ((), ())),
                                         preferred_element_type=F32)
                sc = jnp.where(mask, sc, -1e9 / scale)
                p = jnp.exp2((sc - jnp.max(sc, axis=-1, keepdims=True)) * (scale * LOG2E))
                P[hd] = p
                Z[hd] = jnp.sum(p, axis=-1, keepdims=True)
            elif op == "P":
                z = Z.pop(hd)
                r = pltpu.reciprocal(z, approx=True)
                r = r * (2.0 - z * r)
                O[hd] = jnp.dot(P.pop(hd), V.pop(hd), preferred_element_type=F32) * r
            else:
                if first and hd % HPP == 0:
                    wo_copy(hd // HPP).wait()
                    if hd // HPP + WO_DEPTH < NCT:
                        wo_copy(hd // HPP + WO_DEPTH).start()
                    if hd == H - HPP:
                        for cp in first_block_copies(1):
                            cp.start()
                o = O.pop(hd)
                for nn in range(NT):
                    cols = slice(nn * LANES, (nn + 1) * LANES)
                    y = jnp.dot(o, wo[hd * E:(hd + 1) * E, cols], preferred_element_type=F32)
                    if hd == 0:
                        accb[:, cols] = y
                    elif hd < H - 1:
                        accb[:, cols] += y
                    else:
                        acc[nn] = accb[:, cols] + y
        for fn in side.pop(len(ops), []):
            fn()
        out = jnp.concatenate(acc, axis=1).astype(BF16)
        hbuf[0:M, :] = out[0:M].astype(F32)
        abuf[pl.ds(r0, SEG), :] = out[M:L]
        send_outputs(s, c, part)
        nxt = s + 1

        @pl.when((nxt % SPT == 0) & (nxt < NSEG))
        def _():
            wait_block_inputs(nxt // SPT)

        if fast:
            @pl.when(nxt == EARLY)
            def _():
                for cp in first_block_copies(1):
                    cp.wait()
                start_late()

    for cp in first_block_copies(0):
        cp.wait()
    segment(0, first=True)
    jax.lax.fori_loop(1, NPRE + 1, lambda s, z: (segment(s, fast=True), z)[1], 0)
    jax.lax.fori_loop(NPRE + 1, NSEG, lambda s, z: (segment(s), z)[1], 0)

    pltpu.make_async_copy(qb, qb, sem_ob).wait()
    pltpu.make_async_copy(abuf, out_hbm.at[:, pl.ds(0, DM)], sem_a).wait()


@functools.partial(jax.jit, static_argnames=("A_seg_len",))
def pallas_concat_heads__memory_aug_recurrent_mem_tr__ssm_conv_h3__prompt_kernel(
    A_x: jax.Array,
    A_mem0: jax.Array,
    A_Wq: jax.Array,
    A_Wk: jax.Array,
    A_Wv: jax.Array,
    A_Wo: jax.Array,
    A_seg_len: int,
    B_q: jax.Array,
    B_k: jax.Array,
    B_v: jax.Array,
    B_shift_k: jax.Array,
    B_ssm_k: jax.Array,
    B_ssm_D: jax.Array,
):
    B, S, DM = A_x.shape
    H, E = A_Wq.shape[1], A_Wq.shape[2]
    M = A_mem0.shape[1]
    SEG = int(A_seg_len)
    D = B_q.shape[2]
    KS = B_shift_k.shape[1]
    NCT = D // LANES
    NCH = S // CHUNK
    DCH = DM // NCT
    NSEG = S // SEG
    assert B == 1 and E == LANES and M == 8 and KS <= 8
    assert S % CHUNK == 0 and S % SEG == 0 and NSEG % NCT == 0 and NCH % (NSEG // NCT) == 0
    assert H % NCT == 0 and DCH % 16 == 0 and (CHUNK // 8) % (NSEG // NCT) == 0
    CPS = NCH // (NSEG // NCT)
    NSP = NCH * 2 * CHUNK // (DM // 2)

    kernel = functools.partial(_kernel, S=S, DM=DM, H=H, E=E, M=M, SEG=SEG, D=D, KS=KS)
    hbm = pl.BlockSpec(memory_space=pl.ANY)
    dma = pltpu.SemaphoreType.DMA

    out = pl.pallas_call(
        kernel,
        out_shape=jax.ShapeDtypeStruct((S, DM + D), BF16),
        in_specs=[hbm] * 14,
        out_specs=hbm,
        scratch_shapes=[
            pltpu.VMEM((3 * H + 2 * NSP, DM // 2, E), U32),
            pltpu.VMEM((H * E, DM), BF16),
            pltpu.VMEM((NSLOT, DCH * (H // 2), E), U32),
            pltpu.VMEM((S, DM), BF16),
            pltpu.VMEM((S, DM), BF16),
            pltpu.VMEM((M + SEG, DM), F32),
            pltpu.VMEM((M + SEG, DM), F32),
            pltpu.VMEM((2, NPRE * SEG, H * E), BF16),
            pltpu.VMEM((S, D), BF16),
            pltpu.VMEM((S, D), BF16),
            pltpu.VMEM((S, D), BF16),
            pltpu.VMEM((D, S), BF16),
            pltpu.VMEM((2, 8 + CPS * CHUNK, LANES), F32),
            pltpu.VMEM((4, 2 * CHUNK, LANES), F32),
            pltpu.VMEM((2, NCH, 2 * CHUNK, LANES), F32),
            pltpu.VMEM((2, NCH, 2 * CHUNK, LANES), F32),
            pltpu.VMEM((2, NCH, 2 * CHUNK, LANES), F32),
            pltpu.VMEM((M, DM), BF16),
            pltpu.VMEM((KS, D), BF16),
            pltpu.VMEM((NCT, LANES), BF16),
            pltpu.VMEM((2 * CHUNK, CHUNK), BF16),
            pltpu.VMEM((CHUNK, 2 * CHUNK), BF16),
            dma((5,)),
            pltpu.VMEM((NCT, LANES), F32),
            dma((NSLOT,)), dma((NCT,)), dma((NCT + 2,)), dma((NCT + 2,)), dma((NCT + 2, 3)),
            dma, dma,
        ],
        compiler_params=pltpu.CompilerParams(
            vmem_limit_bytes=124 * 1024 * 1024, disable_bounds_checks=True),
    )(
        A_mem0.reshape(M, DM), B_shift_k.T, B_ssm_D.reshape(NCT, LANES),
        jnp.asarray(_FWD, BF16), jnp.asarray(_INV, BF16),
        A_x.reshape(S, DM),
        A_Wq.reshape(DM * H, E), A_Wk.reshape(DM * H, E), A_Wv.reshape(DM * H, E),
        A_Wo.reshape(H * E, DM),
        B_q.reshape(S, D), B_k.reshape(S, D), B_v.reshape(S, D), B_ssm_k,
    )
    return out.reshape(B, S, DM + D)
```
